```python
import os as _os
_os.environ.setdefault('JAX_PLATFORMS', 'cpu')
import jax
import jax.numpy as jnp

def _softmax(x, axis=-1):
    return jax.nn.softmax(x, axis=axis)

def _gelu(x):
    return jax.nn.gelu(x, approximate=True)

def _silu(x):
    return jax.nn.silu(x)

def _sigmoid(x):
    return jax.nn.sigmoid(x)

def _layernorm(x, axis=-1, eps=1e-05):
    m = jnp.mean(x, axis=axis, keepdims=True)
    v = jnp.var(x, axis=axis, keepdims=True)
    return (x - m) / jnp.sqrt(v + eps)

def _scatter_add(tgt, idx, src, axis=0):
    return tgt.at[idx].add(src)

def _segment_sum(src, seg, n):
    return jax.ops.segment_sum(src, seg, n)

class _Rng:

    def __init__(self, key):
        self._k = key

    def _next(self):
        self._k, sub = jax.random.split(self._k)
        return sub

    def normal(self, shape):
        return jax.random.normal(self._next(), shape, dtype=jnp.bfloat16)

    def randint(self, lo, hi, shape):
        return jax.random.randint(self._next(), shape, lo, hi, dtype=jnp.int32)

    def uniform(self, shape, lo=0.0, hi=1.0):
        return jax.random.uniform(self._next(), shape, jnp.bfloat16, lo, hi)

    def permutation(self, n):
        return jax.random.permutation(self._next(), n)
kernel_name = 'concat_heads__spectral_gfnet__memory_aug_recurrent_mem_tr__prompt'

def setup_inputs():
    _rng = _Rng(jax.random.key(int.from_bytes(__import__("os").urandom(4), "little")))
    _w = lambda a: (lambda t: t.astype(jnp.bfloat16) if jnp.issubdtype(t.dtype, jnp.floating) else t)(jnp.asarray(a))

    def _A_setup():
        B, S, D = (1, 2048, 512)
        Df = D // 2 + 1
        return {'x': _w((lambda *s: _rng.normal(s) * 0.05)(B, S, D)), 'w_r': _w((lambda *s: _rng.normal(s) * 0.05)(S, Df) * 0.02), 'w_i': _w((lambda *s: _rng.normal(s) * 0.05)(S, Df) * 0.02)}
    _A_in = _A_setup()

    def _B_setup():
        B, S, Dm = (1, 2048, 512)
        H, Dh = (32, 128)
        M, seg = (8, 32)
        seg = min(seg, S)
        S = S // seg * seg
        return {'x': _w((lambda *s: _rng.normal(s) * 0.05)(B, S, Dm)), 'mem0': _w((lambda *s: _rng.normal(s) * 0.4)(B, M, Dm)), 'Wq': _w((lambda *s: _rng.normal(s) * 3.2)(Dm, H, Dh) * Dm ** (-0.5)), 'Wk': _w((lambda *s: _rng.normal(s) * 3.2)(Dm, H, Dh) * Dm ** (-0.5)), 'Wv': _w((lambda *s: _rng.normal(s) * 0.4)(Dm, H, Dh) * Dm ** (-0.5)), 'Wo': _w((lambda *s: _rng.normal(s) * 0.4)(H, Dh, Dm) * (H * Dh) ** (-0.5)), 'seg_len': seg}
    _B_in = _B_setup()
    return {'A_x': _A_in['x'], 'A_w_r': _A_in['w_r'], 'A_w_i': _A_in['w_i'], 'B_x': _B_in['x'], 'B_mem0': _B_in['mem0'], 'B_Wq': _B_in['Wq'], 'B_Wk': _B_in['Wk'], 'B_Wv': _B_in['Wv'], 'B_Wo': _B_in['Wo'], 'B_seg_len': _B_in['seg_len']}

def reference(A_x, A_w_r, A_w_i, B_x, B_mem0, B_Wq, B_Wk, B_Wv, B_Wo, B_seg_len):

    def _A_ref(x, w_r, w_i):
        B, S, D = x.shape
        X = (lambda x, axes=(-2, -1): jnp.fft.rfft2(x.astype(jnp.float32), axes=axes))(x, axes=(-2, -1))
        W = w_r + 1j * w_i
        X = X * W
        y = (lambda x, s, axes=(-2, -1): jnp.fft.irfft2(x, s=s, axes=axes).astype(jnp.bfloat16))(X, (S, D), axes=(-2, -1))
        return y

    def _B_ref(x, mem0, Wq, Wk, Wv, Wo, seg_len):
        B, S, Dm = x.shape
        H, Dh = (Wq.shape[1], Wq.shape[2])
        M = mem0.shape[1]
        scale = Dh ** (-0.5)
        n_seg = S // seg_len
        L = M + seg_len
        idx = jnp.arange(L)
        mask = (idx[:, None] < M) | (idx[:, None] >= idx[None, :])
        mem = mem0
        outs = []
        for s in range(n_seg):
            xs = x[:, s * seg_len:(s + 1) * seg_len, :].copy()
            h = jnp.concatenate([mem, xs], axis=1)
            q = jnp.einsum('btd,dhe->bhte', h, Wq)
            k = jnp.einsum('btd,dhe->bhte', h, Wk)
            v = jnp.einsum('btd,dhe->bhte', h, Wv)
            scores = jnp.einsum('bhqe,bhke->bhqk', q, k) * scale
            scores = jnp.where(mask[None, None], scores, -1000000000.0)
            p = _softmax(scores, axis=-1)
            o = jnp.einsum('bhqk,bhke->bhqe', p, v)
            o = jnp.einsum('bhte,hed->btd', o, Wo)
            mem = o[:, :M, :].copy()
            outs.append(o[:, M:, :])
        return jnp.concatenate(outs, axis=1)
    a = _A_ref(A_x, A_w_r, A_w_i)
    b = _B_ref(B_x, B_mem0, B_Wq, B_Wk, B_Wv, B_Wo, B_seg_len)
    return jnp.concatenate([a, b], axis=-1)
```

```python
import jax
import jax.numpy as jnp
import numpy as np
from jax import lax
import jax.experimental.pallas as pl
import jax.experimental.pallas.tpu as pltpu

F32, BF16, U32 = jnp.float32, jnp.bfloat16, jnp.uint32
NN = (((1,), (0,)), ((), ()))
NT = (((1,), (1,)), ((), ()))

S, D = 2048, 512
M, SEG, H, DH = 8, 32, 32, 128
L = M + SEG
NSEG = S // SEG
LOG2E = 1.4426950408889634

STEPS = 8
LATE = 3
PAIRS = 3 * H // 2
PHASES = ((0, 2, 1), (2, 4, 3), (14, 5, 2), (24, 12, 2))
ORDER_FORWARD = ("PPOOPOOOTTOOTOTPTOOTOOOTTPTTTTOOPOPPTTPPPPTTPPPPPPPPSPPPSPSPSPPSPPSPPPPPPSPSPSPPSPPSPPPSPPSPPSPPPPSPSPPP"
                 "SPSPPPPPPPPPPPPP")
ORDER_FILTER = 2 * ("PPFPFPFPFPPFPPFPPFPPFPFPPFPPFPFPPFPPFPPFPPFPPPFPFPFPFPPFPPFPPFPPFPPFPFPPFPFPPPFPFPPFPPFPFPPFPPFP"
                    "FPPFPPFPPFPPFPPFPPFPFPFPPPFPFPPFPPFP")
SPEC = 3 * H * D // 2
NYQ = 16 * 512
ZERO = SPEC + NYQ + 256


def _dft_constants():
    d = np.arange(128)
    j = (8 * np.arange(8)[:, None] + np.array([0, 4, 1, 5, 2, 6, 3, 7])[None, :]).reshape(-1)

    def cos_sin(r):
        ang = 2 * np.pi * (np.outer(4 * j + r, d) % D) / D
        return np.cos(ang), np.sin(ang)

    (c0, s0), (c1, s1), (c2, s2), (c3, s3) = [cos_sin(r) for r in range(4)]
    f0 = np.concatenate([c0, -s0])
    f0[64] = 1.0 - 2.0 * (d % 2)
    row = np.arange(128)
    cos, sin = np.concatenate([c1, c3])[:, :64], np.concatenate([s1, s3])[:, :64]
    sign = np.where(row < 64, -1.0, 1.0)[:, None]
    real, imag = np.concatenate([cos, sign * sin], axis=1), np.concatenate([-sin, sign * cos], axis=1)[row ^ 2]
    own = (((row & 2) == 0) == (row < 64))[:, None]
    fd = np.stack([f0, np.concatenate([c2, -s2]), np.where(own, real, imag), np.where(own, imag, real),
                   np.concatenate([-s2, c2])])
    i, u, half, sigma, t1, f1 = np.ix_(*[np.arange(n) for n in (2, 4, 2, 2, 64, 64)])
    ang = 2 * np.pi * (((32 * t1 + 16 * sigma + 4 * u + 2 * i + half) * f1) % S) / S
    gr, gi = np.cos(ang), -np.sin(ang)
    g = np.concatenate([np.concatenate([gr, gi], axis=-1), np.concatenate([-gi, gr], axis=-1)], axis=-2)
    ang = 2 * np.pi * np.arange(16)[:, None, None] / 32
    low = np.arange(128)[None, None, :] < 64
    turns = np.concatenate([np.cos(ang) * np.ones_like(low), np.where(low, -np.sin(ang), np.sin(ang)),
                            np.zeros((16, 6, 128))], axis=1)
    return fd.astype(np.float32).astype(BF16), g.astype(np.float32).astype(BF16), turns.astype(np.float32)


_FD, _G, _TURNS = _dft_constants()
_INDICES = np.arange(128, dtype=np.int32) ** 2
_C8, _S8, _R2 = float(np.cos(np.pi / 8)), float(np.sin(np.pi / 8)), float(np.sqrt(0.5))

_PRODUCTS = (
    (((0, 0), (1, 1), 1), ((0, 0), (1, 1), 1), (((0, 0), 1), ((1, 1), 1))),
    (((1, 0), (1, 1), 1), ((0, 0),), (((1, 0), 1), ((1, 1), -1))),
    (((1, 1),), ((1, 0), (0, 0), -1), (((0, 0), 1), ((1, 0), 1))),
    (((0, 0), (0, 1), 1), ((1, 1),), (((0, 0), -1), ((0, 1), 1))),
    (((0, 1), (1, 1), -1), ((1, 0), (1, 1), 1), (((0, 0), 1),)),
    (((0, 0),), ((0, 1), (1, 1), -1), (((0, 1), 1), ((1, 1), 1))),
    (((1, 0), (0, 0), -1), ((0, 0), (0, 1), 1), (((1, 1), 1),)),
)


def _dot(a, b, dims=NN):
    return lax.dot_general(a, b, dims, preferred_element_type=F32)


def _radix4(a, b, c, d, sign):
    t0 = (a[0] + c[0], a[1] + c[1])
    t1 = (a[0] - c[0], a[1] - c[1])
    t2 = (b[0] + d[0], b[1] + d[1])
    t3 = (b[0] - d[0], b[1] - d[1])
    y0 = (t0[0] + t2[0], t0[1] + t2[1])
    y2 = (t0[0] - t2[0], t0[1] - t2[1])
    ya = (t1[0] + t3[1], t1[1] - t3[0])
    yb = (t1[0] - t3[1], t1[1] + t3[0])
    return (y0, ya, y2, yb) if sign < 0 else (y0, yb, y2, ya)


def _twiddle16(z, e):
    re, im = z
    if e == 0:
        return z
    if e == 4:
        return -im, re
    if e == 2:
        return (re - im) * _R2, (im + re) * _R2
    if e == 6:
        return (re + im) * (-_R2), (re - im) * _R2
    c, s = {1: (_C8, _S8), 3: (_S8, _C8), 9: (-_C8, -_S8)}[e]
    return re * c - im * s, im * c + re * s


def _lo(w):
    return pltpu.bitcast(w << 16, F32)


def _hi(w):
    return pltpu.bitcast(w & np.uint32(0xFFFF0000), F32)


def _pack(even, odd):
    return pltpu.bitcast(pltpu.pack_elementwise([even, odd], packed_dtype=BF16), U32)


def _kernel(ax_hbm, wr_hbm, wi_hbm, bx_hbm, mem_hbm, wq_hbm, wk_hbm, wv_hbm, wo_hbm, fd_hbm, g_hbm, turns_hbm,
            idx_hbm, out_hbm,
            ax, wr, wi, wr_last, wi_last, fd, gt, turns, ybuf, work, ya, raw, xs, wo, xpre, xrest, mem0, pre, yb, idx,
            sems):
    ax32 = ax_hbm.bitcast(U32)
    wo32 = wo_hbm.bitcast(U32)
    out32 = out_hbm.bitcast(U32)
    w32 = [w.bitcast(U32) for w in (wq_hbm, wk_hbm, wv_hbm)]

    sem_phase = [1 + sum(p[2] for p in PHASES[:n]) for n in range(5)]
    sem_fd, sem_filter, sem_rest = [sem_phase[4] + n for n in range(3)]

    def pairs(phase, i):
        first, count, _ = PHASES[phase]
        return [(w32[p // 16].at[:, p % 16, :], raw.at[p], sem_phase[phase] + i)
                for p in range(first + count * i, first + count * (i + 1))]

    def filters(src, dst, last):
        return [(src.at[pl.ds(0, D // 2)].bitcast(U32), dst, sem_filter), (src.at[pl.ds(D // 2, 1)], last, sem_filter)]

    plan = [(idx_hbm, idx, 0), (bx_hbm.at[:, pl.ds(0, 8), :], xpre, 0)] + pairs(0, 0)
    for i in range(PHASES[1][2]):
        plan += pairs(1, i)
    plan += [(fd_hbm, fd, sem_fd)]
    for i in range(2):
        plan += pairs(2, i)
        plan += [(ax32.at[:, 8 * sigma + c, :], ax.at[c, sigma], sem_phase[2] + i)
                 for c in range(i, 8, 2) for sigma in range(2)]
        plan += [(g_hbm.at[i], gt.at[i], sem_phase[2] + i)]
    plan += filters(wr_hbm, wr, wr_last) + filters(wi_hbm, wi, wi_last)
    for i in range(PHASES[3][2]):
        plan += pairs(3, i)
    plan += [(turns_hbm, turns, sem_rest), (mem_hbm, mem0, sem_rest),
             (bx_hbm.at[:, pl.ds(8, SEG - 8), :], xrest, sem_rest)]
    plan += [(wo32.at[:, pl.ds(128 * j, 128)], wo.at[j], sem_rest) for j in range(4)]
    for src, dst, sem in plan:
        pltpu.make_async_copy(src, dst, sems.at[sem]).start()

    def wait(sem):
        for src, dst, n in plan:
            if n == sem:
                pltpu.make_async_copy(src, dst, sems.at[sem]).wait()

    def wait_for(dst, sem):
        pltpu.make_async_copy(dst, dst, sems.at[sem]).wait()

    sub = lax.broadcasted_iota(jnp.int32, (8, 128), 0)
    lane = lax.broadcasted_iota(jnp.int32, (264, 128), 1)
    low = lane < 64
    row0 = sub == 0

    def rows(base, off, n):
        return pl.ds((base if isinstance(base, int) else pl.multiple_of(base, 32)) + off, n)

    def pinned(base, off, n):
        return rows(idx[0] + base, off, n)

    work[pl.ds(ZERO, 8), :] = jnp.zeros((8, 128), U32)

    def after_stores(words):
        return jnp.concatenate([words[:8] | work[pinned(ZERO, 0, 8), :], words[8:]], axis=0)

    def get(where):
        return pltpu.bitcast(work[where, :], F32)

    def put(where, v):
        work[where, :] = pltpu.bitcast(v, U32)

    fw = {}

    def by_group(v):
        return jnp.concatenate([v[64 * blk + 8 * jg:64 * blk + 8 * jg + 8] for jg in range(8) for blk in range(4)], 0)

    def by_block(v):
        return jnp.concatenate([v[32 * jg + 8 * blk:32 * jg + 8 * blk + 8] for blk in range(4) for jg in range(8)], 0)

    def a_features(i, u, n):
        if n == 0:
            words = [jnp.concatenate([ax[i + 2 * u, sigma, :, 128 * j:128 * (j + 1)] for sigma in range(2)], axis=0)
                     for j in range(4)]
            x = [jnp.concatenate([_lo(w), _hi(w)], axis=0) for w in words]
            a0, a1, b0, b1 = x[0] + x[2], x[1] + x[3], x[0] - x[2], x[1] - x[3]
            base = jnp.where(low[:256], b0, pltpu.roll(b1, 64, 1))
            t = jnp.where(low[:256], pltpu.roll(b0 - b1, 64, 1), b0 + b1) * _R2
            fw[u] = [v.astype(BF16) for v in (a0 + a1, a0 - a1, base + t, base - t)]
        fw[u][n] = _dot(fd[n], fw[u][n], NT)

    def a_time(i, u, half, sigma):
        if half == 0 and sigma == 0:
            e0, e2, qa, qb = fw[u]
            first = jnp.concatenate([(sub & 2) == 0] * 2, axis=1)
            re, im = [], []
            for r in range(0, 128, 8):
                x, y = (qa[r:r + 8], qb[r:r + 8]) if r < 64 else (qb[r:r + 8], qa[r:r + 8])
                re.append(jnp.where(first, x, y))
                t = jnp.where(first, y, x)
                im.append(jnp.where(first, pltpu.roll(t, 6, 0), pltpu.roll(t, 2, 0)))
            nyq = e0[64:72]
            fw[u] = (jnp.concatenate([e0[:64], e2[:64]] + re + [nyq], axis=0),
                     jnp.concatenate([jnp.where(jnp.concatenate([row0, row0], axis=1), 0.0, nyq), e0[72:], e2[64:]]
                                     + im + [jnp.zeros_like(nyq)], axis=0))
        g = gt[i, u, half, sigma]
        if sigma == 0:
            xr, xi = [v[:, 128 * half:128 * (half + 1)] for v in fw[u]]
            xi = pltpu.roll(xi, 64, 1)
            fw["odd"] = jnp.where(low, xi, xr)
            fw["even"] = _dot(jnp.where(low, xr, xi), g)
            return
        odd = _dot(fw["odd"], jnp.concatenate([g[64:], g[:64]], axis=0))
        total, diff = fw["even"] + odd, fw["even"] - odd
        c, s = [jnp.where(i == 0, f(2 * np.pi * (4 * u + half) / 32), f(2 * np.pi * (4 * u + half + 2) / 32)).astype(F32)
                for f in (np.cos, np.sin)]
        other = pltpu.roll(diff, 64, 1)
        for d, y in enumerate((jnp.where(low, total, c * other + s * diff),
                               jnp.where(low, pltpu.roll(total, 64, 1), c * diff - s * other))):
            ybuf[rows(1024 * i, 2048 * u + 512 * half + 256 * d, 256), :] = by_group(y[:256])
            ybuf[rows(32 * i, NYQ + 64 * u + 16 * half + 8 * d, 8), :] = y[256:]

    def a_spread(i, half, jg):
        tw = [[jnp.where(i == 0, f(2 * np.pi * half * k / 16), f(2 * np.pi * (2 + half) * k / 16)).astype(F32)
               for f in (np.cos, np.sin)] for k in range(4)]
        if jg == 8:
            todo = [[(32 * i, NYQ + 64 * u + 16 * half, 8) for u in range(4)]]
        else:
            todo = [[(1024 * i, 2048 * u + 512 * half + 32 * jg + 8 * blk, 256) for u in range(4)] for blk in range(4)]
        for slots in todo:
            x = _radix4(*[(ybuf[pinned(b, o, 8), :], ybuf[pinned(b, o + d, 8), :]) for b, o, d in slots], -1)
            for k, ((b, o, d), (re, im)) in enumerate(zip(slots, x)):
                if k > 0:
                    c, s = tw[k]
                    re, im = re * c + im * s, im * c - re * s
                put(rows(b, SPEC + o, 8), re)
                put(rows(b, SPEC + o + d, 8), im)

    def weight(i, jg, blk, f):
        cols = slice(128 * f, 128 * (f + 1))
        if blk == 4:
            return tuple(jnp.broadcast_to(r[:, cols].astype(F32) * 0.5, (8, 128)) for r in (wr_last, wi_last))
        out = []
        for r in (wr, wi):
            v = r[rows(64 * i, 16 * jg, 16), cols]
            if blk % 2 == 0:
                v = jnp.where(sub % 2 == 0, v[:8], pltpu.roll(v[8:], 1, 0))
            else:
                v = jnp.where(sub % 2 == 0, pltpu.roll(v[:8], 7, 0), v[8:])
            v = _lo(v) if blk < 2 else _hi(v)
            if blk == 0 and jg == 0:
                v = v * jnp.where(jnp.logical_and(row0, i == 0), 0.5, 1.0).astype(F32)
            out.append(v)
        return tuple(out)

    def slot(jg, blk, s):
        if blk == 4:
            return SPEC + NYQ + 16 * s, SPEC + NYQ + 16 * s + 8
        return SPEC + 512 * s + 32 * jg + 8 * blk, SPEC + 512 * s + 256 + 32 * jg + 8 * blk

    def a_filter(i, jg, blk, t):
        slots = [slot(jg, blk, 4 * t + u) for u in range(4)]
        x = _radix4(*[tuple(get(pinned(128 * i, r, 8)) for r in ri) for ri in slots], -1)
        w = [weight(i, jg, blk, t + 4 * k) for k in range(4)]
        x = [(v[0] * u[0] - v[1] * u[1], v[0] * u[1] + v[1] * u[0]) for v, u in zip(x, w)]
        for n, (ri, v) in enumerate(zip(slots, _radix4(*x, +1))):
            v = _twiddle16(v, t * n)
            put(rows(128 * i, ri[0], 8), v[0])
            put(rows(128 * i, ri[1], 8), v[1])

    def a_gather(i, jg, blk, ts):
        todo = [[slot(jg, blk, 4 * u + t) for u in range(4)] for t in ts]
        values = [[tuple(get(pinned(128 * i, r, 8)) for r in ri) for ri in slots] for slots in todo]
        for slots, x in zip(todo, values):
            for ri, v in zip(slots, _radix4(*x, +1)):
                put(rows(128 * i, ri[0], 8), v[0])
                put(rows(128 * i, ri[1], 8), v[1])

    def filter_work(i, jg, blk):
        return [(a_filter, (i, jg, blk, t)) for t in range(4)] + [(a_gather, (i, jg, blk, ts)) for ts in ((0, 1), (2, 3))]

    def a_inverse_time(c):
        zr, zi = [], []
        for half in range(2):
            ur, ui = [jnp.concatenate([by_block(get(rows(1024 * c, SPEC + 512 * half + 256 * d, 256))),
                                       get(rows(32 * c, SPEC + NYQ + 16 * half + 8 * d, 8))], axis=0)
                      for d in range(2)]
            co, si = turns[2 * c + half, 0:1], turns[2 * c + half, 1:2]
            moved = pltpu.roll(ui, 64, 1)
            base = jnp.where(low, ur, moved)
            t = co * jnp.where(low, pltpu.roll(ur, 64, 1), ui) + si * jnp.where(low, moved, ur)
            for sigma, v in enumerate((base + t, base - t)):
                g = gt[c % 2, c // 2, half, sigma]
                k = _dot(g, v[:256].astype(BF16), NT)
                nyq = jnp.sum(g[:64].astype(F32) * v[256:257], axis=1, keepdims=True)
                zr.append(k[:64])
                zi.append(jnp.concatenate([jnp.where(lane[:64] == 0, nyq, k[64:, :128]), k[64:, 128:]], axis=1))
        return jnp.concatenate(zr, axis=0), jnp.concatenate(zi, axis=0)

    def a_inverse_features(c, zr, zi):
        lo = low[:256]
        rot = pltpu.roll(zi[:, :128], 64, 1)
        u0 = _dot(jnp.where(lo, zr[:, :128], rot), fd[0])
        u2 = _dot(jnp.where(lo, rot, zr[:, :128]), fd[4])
        zr, zi = zr[:, 128:], zi[:, 128:]
        first = (lane[:256] & 2) == 0
        own = first == lo
        zi = jnp.where(first, pltpu.roll(zi, 126, 1), pltpu.roll(zi, 2, 1))
        wa, wb = _dot(jnp.where(own, zr, zi), fd[2]), _dot(jnp.where(own, zi, zr), fd[3])
        total, diff = wa + wb, wa - wb
        other = pltpu.roll(diff, 64, 1)
        v0 = jnp.where(lo, total, (other + diff) * _R2)
        v1 = jnp.where(lo, pltpu.roll(total, 64, 1), (diff - other) * _R2)
        e0, e1 = u0 + u2, u0 - u2
        for j, y in enumerate((e0 + v0, e1 + v1, e0 - v0, e1 - v1)):
            y = y * (2.0 / (S * D))
            y = _pack(y[:128], y[128:])
            for sigma in range(2):
                ya[c, j, pl.ds(sigma, 64, stride=2), :] = y[64 * sigma:64 * (sigma + 1)]

    part = {}

    def combine(spec, block):
        return _pack(*[a + b if spec[2] > 0 else a - b for a, b in zip(block(*spec[0]), block(*spec[1]))])

    def early(p, n, mc):
        def words(r):
            return [raw[p, pl.ds(D // 2 * r + odd, D // 4, stride=2), :] for odd in range(2)]

        _, right, uses = _PRODUCTS[n]
        x = xs[n, (pinned if isinstance(p, int) else rows)(0, 64 * mc, 64), :]
        if mc == 1:
            x = jnp.concatenate([after_stores(x[:, :128]), x[:, 128:]], axis=1)
        elif len(right) > 1:
            part["w"] = after_stores(combine(right, lambda r, c: [(_lo, _hi)[c](w) for w in words(r)]))
        else:
            r, c = right[0]
            a, b = words(r)
            plain = (a & np.uint32(0xFFFF)) | (b << 16), (a >> 16) | (b & np.uint32(0xFFFF0000))
            part["w"] = after_stores(plain[c])
            for h in range(2):
                work[rows(p * D, h * (D // 2) + r * (D // 4), D // 4), :] = plain[h]
        prod = _dot(pltpu.bitcast(x, BF16), pltpu.bitcast(part["w"], BF16))
        for key, sign in uses:
            total, count = part.pop((key, mc), (None, 0))
            total = prod if total is None else (total + prod if sign > 0 else total - prod)
            if count + 1 == (4 if key[0] == key[1] else 2):
                pre[rows(p * 16 * NSEG, key[1] * 8 * NSEG + 4 * NSEG * key[0] + 128 * mc, 128), :] = total
            else:
                part[key, mc] = total, count + 1

    def early_work(phase, i):
        first, count, _ = PHASES[phase]
        wait_for(raw.at[pl.ds(first + count * i, count)], sem_phase[phase] + i)
        return [(early, (first + count * i + u, n, mc)) for u in range(count) for n in range(7) for mc in range(2)]

    def run(order, **queues):
        for name in order:
            fn, args = queues[name].pop(0)
            fn(*args)
        assert not any(queues.values())

    def plain_phase(phase, i):
        todo = early_work(phase, i)
        run("P" * len(todo), P=todo)

    def forward_phase(i):
        wait_for(ax.at[pl.ds(0, 4)], sem_phase[2] + i)
        wait_for(gt.at[i], sem_phase[2] + i)
        run(ORDER_FORWARD, P=early_work(2, i),
            O=[(a_features, (i, u, n)) for u in range(4) for n in range(4)],
            T=[(a_time, (i, u, half, sigma)) for u in range(4) for half in range(2) for sigma in range(2)],
            S=[(a_spread, (i, half, jg)) for jg in range(9) for half in range(2)])

    def filter_phase(i):
        run(ORDER_FILTER, P=early_work(3, i), F=[w for jg in range(4) for blk in range(4) for w in filter_work(i, jg, blk)])

    wait(0)
    xp = pltpu.bitcast(xpre[...].reshape(8 * NSEG, D), U32)

    def rows_of_x(r, c):
        return xp[128 * r:128 * (r + 1), 256 * c:256 * (c + 1)]

    for n, (left, _, _) in enumerate(_PRODUCTS):
        if len(left) == 1:
            xs[n] = rows_of_x(*left[0])
        else:
            xs[n] = combine(left, lambda r, c: [f(rows_of_x(r, c)) for f in (_lo, _hi)])
    plain_phase(0, 0)
    pl.loop(0, PHASES[1][2])(lambda i: plain_phase(1, i))
    wait(sem_fd)
    pl.loop(0, 2)(forward_phase)
    wait(sem_filter)
    run("F" * 6, F=filter_work(0, 0, 4))
    pl.loop(0, 2)(filter_phase)
    wait(sem_rest)

    row = lax.broadcasted_iota(jnp.int32, (L, L), 0)
    col = lax.broadcasted_iota(jnp.int32, (L, L), 1)
    mask = (row >= SEG) | (col >= SEG) | (row >= col)
    scale = DH ** -0.5

    def w_in(i, g):
        return jnp.concatenate(
            [pltpu.bitcast(work[pl.ds((i * H + 4 * g + j) * (D // 2), D // 2), :], BF16) for j in range(4)], axis=1)

    def w_out(g):
        return jnp.concatenate([pltpu.bitcast(wo[j, 256 * g:256 * (g + 1)], BF16) for j in range(4)], axis=1)

    def step(s, carry):
        mem, late_o, late_acc = carry
        h = jnp.concatenate([xrest[s].astype(F32), mem], axis=0).astype(BF16)
        st = {"late": late_acc}

        def project(i, g):
            known = [pre[pl.ds(pl.multiple_of(s * 8, 8) + (i * H + 4 * g + j) * 8 * NSEG, 8), :] for j in range(4)]
            st[i, g] = jnp.concatenate([jnp.concatenate(known, axis=1), _dot(h, w_in(i, g))], axis=0)

        def softmax(g):
            ps = []
            for j in range(4):
                cols = slice(DH * j, DH * (j + 1))
                sc = _dot(st[0, g][:, cols], st[1, g][:, cols], NT)
                sc = jnp.where(mask, sc * (scale * LOG2E), -1e9 * LOG2E)
                e = jnp.exp2(sc - jnp.max(sc, axis=1, keepdims=True))
                total = jnp.sum(e, axis=1, keepdims=True)
                r = pltpu.reciprocal(total, approx=True)
                ps.append((e, r * (2.0 - total * r)))
            st["p", g] = ps

        def mix_rows(g, which):
            v = st[2, g].astype(BF16)
            return jnp.concatenate([_dot(e[which], v[:, DH * j:DH * (j + 1)]) * r[which]
                                    for j, (e, r) in enumerate(st["p", g])], axis=1)

        def mix(g):
            if g >= 8 - LATE:
                st["o", g] = jnp.concatenate([mix_rows(g, slice(SEG, L)), late_o[g - (8 - LATE)]], axis=0)
            else:
                o = mix_rows(g, slice(0, L))
                st["o", g] = jnp.concatenate([o[SEG:], o[:SEG]], axis=0)

        def output(g):
            r = _dot(st["o", g], w_out(g))
            st["mem"] = r[:M] if g == 0 else st["mem"] + r[:M]
            key = "late" if g >= 8 - LATE else "tokens"
            st[key] = r[M:] if g == 0 else st[key] + r[M:]

        for g in range(8):
            project(1, g)
            project(0, g)
            if g > 0:
                mix(g - 1)
            project(2, g)
            softmax(g)
        output(0)
        output(1)
        mix(7)
        for g in range(2, 8):
            output(g)
        late_o = tuple(mix_rows(g, slice(0, SEG)) for g in range(8 - LATE, 8))
        yb[pl.ds(2 * s, 2)] = st["late"].astype(BF16).reshape(2, 16, D)
        return st["mem"], late_o, st["tokens"]

    def b_out(first, n):
        return pltpu.make_async_copy(
            yb.at[pl.ds(2 * first + 2, 2 * n)], out_hbm.at[pl.ds(2 * first, 2 * n), :, pl.ds(D, D)], sems.at[0])

    def block(i, carry):
        carry = step(i * STEPS, carry)
        z = a_inverse_time(i)
        carry = step(i * STEPS + 1, carry)
        a_inverse_features(i, *z)
        for u in range(2, STEPS):
            carry = step(i * STEPS + u, carry)
        for j in range(4):
            pltpu.make_async_copy(ya.at[i, j], out32.at[:, i, pl.ds(128 * j, 128)], sems.at[0]).start()

        @pl.when(i == 0)
        def _():
            b_out(0, STEPS - 1).start()

        @pl.when(i > 0)
        def _():
            b_out(i * STEPS - 1, STEPS).start()

        return carry

    zeros = jnp.zeros((SEG, D), F32)
    _, late_o, acc = lax.fori_loop(0, NSEG // STEPS, block, (mem0[...].astype(F32), (zeros,) * LATE, zeros))
    for g in range(8 - LATE, 8):
        acc = acc + _dot(late_o[g - (8 - LATE)], w_out(g))
    yb[pl.ds(2 * NSEG, 2)] = acc.astype(BF16).reshape(2, 16, D)
    b_out(NSEG - 1, 1).start()
    wait_for(ya, 0)
    b_out(0, NSEG).wait()


def _forward(A_x, A_w_r, A_w_i, B_x, B_mem0, B_Wq, B_Wk, B_Wv, B_Wo):
    in_hbm = pl.BlockSpec(memory_space=pl.ANY)
    out = pl.pallas_call(
        _kernel,
        out_shape=jax.ShapeDtypeStruct((S // 16, 16, 2 * D), BF16),
        in_specs=[in_hbm] * 13,
        out_specs=in_hbm,
        scratch_shapes=[
            pltpu.VMEM((8, 2, 64, D), U32),
            pltpu.VMEM((D // 4, S), U32),
            pltpu.VMEM((D // 4, S), U32),
            pltpu.VMEM((1, S), BF16),
            pltpu.VMEM((1, S), BF16),
            pltpu.VMEM((5, 128, 128), BF16),
            pltpu.VMEM((2, 4, 2, 2, 128, 128), BF16),
            pltpu.VMEM((16, 8, 128), F32),
            pltpu.VMEM((NYQ + 256, 128), F32),
            pltpu.VMEM((ZERO + 8, 128), U32),
            pltpu.VMEM((8, 4, 128, 128), U32),
            pltpu.VMEM((PAIRS, D, 128), U32),
            pltpu.VMEM((7, 2 * NSEG, D // 2), U32),
            pltpu.VMEM((4, H * DH // 2, 128), U32),
            pltpu.VMEM((NSEG, 8, D), BF16),
            pltpu.VMEM((NSEG, SEG - 8, D), BF16),
            pltpu.VMEM((M, D), BF16),
            pltpu.VMEM((3 * H * 8 * NSEG, DH), F32),
            pltpu.VMEM((2 * NSEG + 2, 16, D), BF16),
            pltpu.SMEM((128,), jnp.int32),
            pltpu.SemaphoreType.DMA((4 + sum(p[2] for p in PHASES),)),
        ],
        compiler_params=pltpu.CompilerParams(vmem_limit_bytes=100 * 1024 * 1024),
    )(A_x.reshape(S // 32, 32, D), A_w_r.T, A_w_i.T, B_x.reshape(NSEG, SEG, D), B_mem0.reshape(M, D),
      B_Wq, B_Wk, B_Wv, B_Wo.reshape(H * DH, D), _FD, _G, _TURNS, _INDICES)
    return out.reshape(1, S, 2 * D)


@jax.jit
def pallas_concat_heads__spectral_gfnet__memory_aug_recurrent_mem_tr__prompt_kernel(
    A_x: jax.Array,
    A_w_r: jax.Array,
    A_w_i: jax.Array,
    B_x: jax.Array,
    B_mem0: jax.Array,
    B_Wq: jax.Array,
    B_Wk: jax.Array,
    B_Wv: jax.Array,
    B_Wo: jax.Array,
    B_seg_len: jax.Array,
):
    del B_seg_len
    return _forward(A_x, A_w_r, A_w_i, B_x, B_mem0, B_Wq, B_Wk, B_Wv, B_Wo)
```

```python
import jax
import jax.numpy as jnp
import numpy as np
from jax import lax
import jax.experimental.pallas as pl
import jax.experimental.pallas.tpu as pltpu

F32, BF16, U32 = jnp.float32, jnp.bfloat16, jnp.uint32
NN = (((1,), (0,)), ((), ()))
NT = (((1,), (1,)), ((), ()))

S, D = 2048, 512
M, SEG, H, DH = 8, 32, 32, 128
L = M + SEG
NSEG = S // SEG
LOG2E = 1.4426950408889634

STEPS = 8
LATE = 3
PAIRS = 3 * H // 2
PHASES = ((0, 2, 1), (2, 4, 3), (14, 5, 2), (24, 12, 2))
ORDER_FORWARD = ("PPOOPOOOTTOOTOTPTOOTOOOTTPTTTTOOPOPPTTPPPPTTPPPPPPPPSPPPSPSPSPPSPPSPPPPPPSPSPSPPSPPSPPPSPPSPPSPPPPSPSPPP"
                 "SPSPPPPPPPPPPPPP")
ORDER_FILTER = 2 * ("PPFPFPFPFPPFPPFPPFPPFPFPPFPPFPFPPFPPFPPFPPFPPPFPFPFPFPPFPPFPPFPPFPPFPFPPFPFPPPFPFPPFPPFPFPPFPPFP"
                    "FPPFPPFPPFPPFPPFPPFPFPFPPPFPFPPFPPFP")
SPEC = 3 * H * D // 2
NYQ = 16 * 512
ZERO = SPEC + NYQ + 256


def _dft_constants():
    d = np.arange(128)
    j = (8 * np.arange(8)[:, None] + np.array([0, 4, 1, 5, 2, 6, 3, 7])[None, :]).reshape(-1)

    def cos_sin(r):
        ang = 2 * np.pi * (np.outer(4 * j + r, d) % D) / D
        return np.cos(ang), np.sin(ang)

    (c0, s0), (c1, s1), (c2, s2), (c3, s3) = [cos_sin(r) for r in range(4)]
    f0 = np.concatenate([c0, -s0])
    f0[64] = 1.0 - 2.0 * (d % 2)
    row = np.arange(128)
    cos, sin = np.concatenate([c1, c3])[:, :64], np.concatenate([s1, s3])[:, :64]
    sign = np.where(row < 64, -1.0, 1.0)[:, None]
    real, imag = np.concatenate([cos, sign * sin], axis=1), np.concatenate([-sin, sign * cos], axis=1)[row ^ 2]
    own = (((row & 2) == 0) == (row < 64))[:, None]
    fd = np.stack([f0, np.concatenate([c2, -s2]), np.where(own, real, imag), np.where(own, imag, real),
                   np.concatenate([-s2, c2])])
    i, u, half, sigma, t1, f1 = np.ix_(*[np.arange(n) for n in (2, 4, 2, 2, 64, 64)])
    ang = 2 * np.pi * (((32 * t1 + 16 * sigma + 4 * u + 2 * i + half) * f1) % S) / S
    gr, gi = np.cos(ang), -np.sin(ang)
    g = np.concatenate([np.concatenate([gr, gi], axis=-1), np.concatenate([-gi, gr], axis=-1)], axis=-2)
    ang = 2 * np.pi * np.arange(16)[:, None, None] / 32
    low = np.arange(128)[None, None, :] < 64
    turns = np.concatenate([np.cos(ang) * np.ones_like(low), np.where(low, -np.sin(ang), np.sin(ang)),
                            np.zeros((16, 6, 128))], axis=1)
    return fd.astype(np.float32).astype(BF16), g.astype(np.float32).astype(BF16), turns.astype(np.float32)


_FD, _G, _TURNS = _dft_constants()
_INDICES = np.arange(128, dtype=np.int32) ** 2
_C8, _S8, _R2 = float(np.cos(np.pi / 8)), float(np.sin(np.pi / 8)), float(np.sqrt(0.5))

_PRODUCTS = (
    (((0, 0), (1, 1), 1), ((0, 0), (1, 1), 1), (((0, 0), 1), ((1, 1), 1))),
    (((1, 0), (1, 1), 1), ((0, 0),), (((1, 0), 1), ((1, 1), -1))),
    (((1, 1),), ((1, 0), (0, 0), -1), (((0, 0), 1), ((1, 0), 1))),
    (((0, 0), (0, 1), 1), ((1, 1),), (((0, 0), -1), ((0, 1), 1))),
    (((0, 1), (1, 1), -1), ((1, 0), (1, 1), 1), (((0, 0), 1),)),
    (((0, 0),), ((0, 1), (1, 1), -1), (((0, 1), 1), ((1, 1), 1))),
    (((1, 0), (0, 0), -1), ((0, 0), (0, 1), 1), (((1, 1), 1),)),
)


def _dot(a, b, dims=NN):
    return lax.dot_general(a, b, dims, preferred_element_type=F32)


def _radix4(a, b, c, d, sign):
    t0 = (a[0] + c[0], a[1] + c[1])
    t1 = (a[0] - c[0], a[1] - c[1])
    t2 = (b[0] + d[0], b[1] + d[1])
    t3 = (b[0] - d[0], b[1] - d[1])
    y0 = (t0[0] + t2[0], t0[1] + t2[1])
    y2 = (t0[0] - t2[0], t0[1] - t2[1])
    ya = (t1[0] + t3[1], t1[1] - t3[0])
    yb = (t1[0] - t3[1], t1[1] + t3[0])
    return (y0, ya, y2, yb) if sign < 0 else (y0, yb, y2, ya)


def _twiddle16(z, e):
    re, im = z
    if e == 0:
        return z
    if e == 4:
        return -im, re
    if e == 2:
        return (re - im) * _R2, (im + re) * _R2
    if e == 6:
        return (re + im) * (-_R2), (re - im) * _R2
    c, s = {1: (_C8, _S8), 3: (_S8, _C8), 9: (-_C8, -_S8)}[e]
    return re * c - im * s, im * c + re * s


def _lo(w):
    return pltpu.bitcast(w << 16, F32)


def _hi(w):
    return pltpu.bitcast(w & np.uint32(0xFFFF0000), F32)


def _pack(even, odd):
    return (even >> 16) | (odd & np.uint32(0xFFFF0000))


def _kernel(ax_hbm, wr_hbm, wi_hbm, bx_hbm, mem_hbm, wq_hbm, wk_hbm, wv_hbm, wo_hbm, fd_hbm, g_hbm, turns_hbm,
            idx_hbm, out_hbm,
            ax, wr, wi, wr_last, wi_last, fd, gt, turns, ybuf, work, ya, raw, xs, wo, xpre, xrest, mem0, pre, yb, idx,
            sems):
    ax32 = ax_hbm.bitcast(U32)
    wo32 = wo_hbm.bitcast(U32)
    out32 = out_hbm.bitcast(U32)
    w32 = [w.bitcast(U32) for w in (wq_hbm, wk_hbm, wv_hbm)]

    sem_phase = [1 + sum(p[2] for p in PHASES[:n]) for n in range(5)]
    sem_fd, sem_filter, sem_rest, sem_a, sem_b, sem_x, sem_g = [sem_phase[4] + n for n in (0, 1, 2, 3, 4, 5, 7)]

    def pairs(phase, i):
        first, count, _ = PHASES[phase]
        return [(w32[p // 16].at[:, p % 16, :], raw.at[p, pl.ds(0, D)], sem_phase[phase] + i)
                for p in range(first + count * i, first + count * (i + 1))]

    def filters(src, dst, last):
        return [(src.at[pl.ds(0, D // 2)].bitcast(U32), dst, sem_filter), (src.at[pl.ds(D // 2, 1)], last, sem_filter)]

    plan = [(idx_hbm, idx, 0), (bx_hbm.at[:, pl.ds(0, 8), :], xpre, 0)] + pairs(0, 0)
    for i in range(PHASES[1][2]):
        plan += pairs(1, i)
    plan += [(fd_hbm, fd, sem_fd)]
    for i in range(2):
        plan += pairs(2, i)
        plan += [(ax32.at[:, 8 * sigma + 2 * u + i, :], ax.at[i, u, sigma], sem_x + i)
                 for u in range(4) for sigma in range(2)]
        plan += [(g_hbm.at[i], gt.at[i], sem_g + i)]
    plan += filters(wr_hbm, wr, wr_last) + filters(wi_hbm, wi, wi_last)
    for i in range(PHASES[3][2]):
        plan += pairs(3, i)
    plan += [(turns_hbm, turns, sem_rest), (mem_hbm, mem0, sem_rest),
             (bx_hbm.at[:, pl.ds(8, SEG - 8), :], xrest, sem_rest)]
    plan += [(wo32.at[:, pl.ds(128 * j, 128)], wo.at[j], sem_rest) for j in range(4)]
    for src, dst, sem in plan:
        pltpu.make_async_copy(src, dst, sems.at[sem]).start()

    def wait(sem):
        for src, dst, n in plan:
            if n == sem:
                pltpu.make_async_copy(src, dst, sems.at[sem]).wait()

    def wait_for(dst, sem):
        pltpu.make_async_copy(dst, dst, sems.at[sem]).wait()

    sub = lax.broadcasted_iota(jnp.int32, (8, 128), 0)
    lane = lax.broadcasted_iota(jnp.int32, (264, 128), 1)
    low = lane < 64
    row0 = sub == 0

    def rows(base, off, n):
        return pl.ds((base if isinstance(base, int) else pl.multiple_of(base, 32)) + off, n)

    def pinned(base, off, n):
        return rows(idx[0] + base, off, n)

    work[pl.ds(ZERO, 8), :] = jnp.zeros((8, 128), U32)

    def after_stores(words):
        return jnp.concatenate([words[:8] | work[pinned(ZERO, 0, 8), :], words[8:]], axis=0)

    def get(where):
        return pltpu.bitcast(work[where, :], F32)

    def put(where, v):
        work[where, :] = pltpu.bitcast(v, U32)

    fw = {}

    def by_group(v):
        return jnp.concatenate([v[64 * blk + 8 * jg:64 * blk + 8 * jg + 8] for jg in range(8) for blk in range(4)], 0)

    def by_block(v):
        return jnp.concatenate([v[32 * jg + 8 * blk:32 * jg + 8 * blk + 8] for blk in range(4) for jg in range(8)], 0)

    def a_features(i, u, n):
        if n == 0:
            words = [jnp.concatenate([ax[i, u, sigma, :, 128 * j:128 * (j + 1)] for sigma in range(2)], axis=0)
                     for j in range(4)]
            x = [jnp.concatenate([_lo(w), _hi(w)], axis=0) for w in words]
            a0, a1, b0, b1 = x[0] + x[2], x[1] + x[3], x[0] - x[2], x[1] - x[3]
            base = jnp.where(low[:256], b0, pltpu.roll(b1, 64, 1))
            t = jnp.where(low[:256], pltpu.roll(b0 - b1, 64, 1), b0 + b1) * _R2
            fw[u] = [v.astype(BF16) for v in (a0 + a1, a0 - a1, base + t, base - t)]
        fw[u][n] = _dot(fd[n], fw[u][n], NT)

    def a_time(i, u, half, sigma):
        if half == 0 and sigma == 0:
            e0, e2, qa, qb = fw[u]
            first = jnp.concatenate([(sub & 2) == 0] * 2, axis=1)
            re, im = [], []
            for r in range(0, 128, 8):
                x, y = (qa[r:r + 8], qb[r:r + 8]) if r < 64 else (qb[r:r + 8], qa[r:r + 8])
                re.append(jnp.where(first, x, y))
                t = jnp.where(first, y, x)
                im.append(jnp.where(first, pltpu.roll(t, 6, 0), pltpu.roll(t, 2, 0)))
            nyq = e0[64:72]
            fw[u] = (jnp.concatenate([e0[:64], e2[:64]] + re + [nyq], axis=0),
                     jnp.concatenate([jnp.where(jnp.concatenate([row0, row0], axis=1), 0.0, nyq), e0[72:], e2[64:]]
                                     + im + [jnp.zeros_like(nyq)], axis=0))
        g = gt[i, u, half, sigma]
        if sigma == 0:
            xr, xi = [v[:, 128 * half:128 * (half + 1)] for v in fw[u]]
            xi = pltpu.roll(xi, 64, 1)
            fw["odd"] = jnp.where(low, xi, xr)
            fw["even"] = _dot(jnp.where(low, xr, xi), g)
            return
        odd = _dot(fw["odd"], jnp.concatenate([g[64:], g[:64]], axis=0))
        total, diff = fw["even"] + odd, fw["even"] - odd
        c, s = [jnp.where(i == 0, f(2 * np.pi * (4 * u + half) / 32), f(2 * np.pi * (4 * u + half + 2) / 32)).astype(F32)
                for f in (np.cos, np.sin)]
        other = pltpu.roll(diff, 64, 1)
        for d, y in enumerate((jnp.where(low, total, c * other + s * diff),
                               jnp.where(low, pltpu.roll(total, 64, 1), c * diff - s * other))):
            ybuf[rows(1024 * i, 2048 * u + 512 * half + 256 * d, 256), :] = by_group(y[:256])
            ybuf[rows(32 * i, NYQ + 64 * u + 16 * half + 8 * d, 8), :] = y[256:]

    def a_spread(i, half, jg):
        tw = [[jnp.where(i == 0, f(2 * np.pi * half * k / 16), f(2 * np.pi * (2 + half) * k / 16)).astype(F32)
               for f in (np.cos, np.sin)] for k in range(4)]
        if jg == 8:
            todo = [[(32 * i, NYQ + 64 * u + 16 * half, 8) for u in range(4)]]
        else:
            todo = [[(1024 * i, 2048 * u + 512 * half + 32 * jg + 8 * blk, 256) for u in range(4)] for blk in range(4)]
        for slots in todo:
            x = _radix4(*[(ybuf[pinned(b, o, 8), :], ybuf[pinned(b, o + d, 8), :]) for b, o, d in slots], -1)
            for k, ((b, o, d), (re, im)) in enumerate(zip(slots, x)):
                if k > 0:
                    c, s = tw[k]
                    re, im = re * c + im * s, im * c - re * s
                put(rows(b, SPEC + o, 8), re)
                put(rows(b, SPEC + o + d, 8), im)

    def weight(i, jg, blk, f):
        cols = slice(128 * f, 128 * (f + 1))
        if blk == 4:
            return tuple(jnp.broadcast_to(r[:, cols].astype(F32) * 0.5, (8, 128)) for r in (wr_last, wi_last))
        out = []
        for r in (wr, wi):
            v = r[rows(64 * i, 16 * jg, 16), cols]
            if blk % 2 == 0:
                v = jnp.where(sub % 2 == 0, v[:8], pltpu.roll(v[8:], 1, 0))
            else:
                v = jnp.where(sub % 2 == 0, pltpu.roll(v[:8], 7, 0), v[8:])
            v = _lo(v) if blk < 2 else _hi(v)
            if blk == 0 and jg == 0:
                v = v * jnp.where(jnp.logical_and(row0, i == 0), 0.5, 1.0).astype(F32)
            out.append(v)
        return tuple(out)

    def slot(jg, blk, s):
        if blk == 4:
            return SPEC + NYQ + 16 * s, SPEC + NYQ + 16 * s + 8
        return SPEC + 512 * s + 32 * jg + 8 * blk, SPEC + 512 * s + 256 + 32 * jg + 8 * blk

    def a_filter(i, jg, blk, t):
        slots = [slot(jg, blk, 4 * t + u) for u in range(4)]
        x = _radix4(*[tuple(get(pinned(128 * i, r, 8)) for r in ri) for ri in slots], -1)
        w = [weight(i, jg, blk, t + 4 * k) for k in range(4)]
        x = [(v[0] * u[0] - v[1] * u[1], v[0] * u[1] + v[1] * u[0]) for v, u in zip(x, w)]
        for n, (ri, v) in enumerate(zip(slots, _radix4(*x, +1))):
            v = _twiddle16(v, t * n)
            put(rows(128 * i, ri[0], 8), v[0])
            put(rows(128 * i, ri[1], 8), v[1])

    def a_gather(i, jg, blk, ts):
        todo = [[slot(jg, blk, 4 * u + t) for u in range(4)] for t in ts]
        values = [[tuple(get(pinned(128 * i, r, 8)) for r in ri) for ri in slots] for slots in todo]
        for slots, x in zip(todo, values):
            for ri, v in zip(slots, _radix4(*x, +1)):
                put(rows(128 * i, ri[0], 8), v[0])
                put(rows(128 * i, ri[1], 8), v[1])

    def filter_work(i, jg, blk):
        return [(a_filter, (i, jg, blk, t)) for t in range(4)] + [(a_gather, (i, jg, blk, ts)) for ts in ((0, 1), (2, 3))]

    def a_inverse_time(c):
        zr, zi = [], []
        for half in range(2):
            ur, ui = [jnp.concatenate([by_block(get(rows(1024 * c, SPEC + 512 * half + 256 * d, 256))),
                                       get(rows(32 * c, SPEC + NYQ + 16 * half + 8 * d, 8))], axis=0)
                      for d in range(2)]
            co, si = turns[2 * c + half, 0:1], turns[2 * c + half, 1:2]
            moved = pltpu.roll(ui, 64, 1)
            base = jnp.where(low, ur, moved)
            t = co * jnp.where(low, pltpu.roll(ur, 64, 1), ui) + si * jnp.where(low, moved, ur)
            for sigma, v in enumerate((base + t, base - t)):
                g = gt[c % 2, c // 2, half, sigma]
                k = _dot(g, v[:256].astype(BF16), NT)
                nyq = jnp.sum(g[:64].astype(F32) * v[256:257], axis=1, keepdims=True)
                zr.append(k[:64])
                zi.append(jnp.concatenate([jnp.where(lane[:64] == 0, nyq, k[64:, :128]), k[64:, 128:]], axis=1))
        return jnp.concatenate(zr, axis=0), jnp.concatenate(zi, axis=0)

    def a_inverse_features(c, zr, zi):
        lo = low[:256]
        rot = pltpu.roll(zi[:, :128], 64, 1)
        u0 = _dot(jnp.where(lo, zr[:, :128], rot), fd[0])
        u2 = _dot(jnp.where(lo, rot, zr[:, :128]), fd[4])
        zr, zi = zr[:, 128:], zi[:, 128:]
        first = (lane[:256] & 2) == 0
        own = first == lo
        zi = jnp.where(first, pltpu.roll(zi, 126, 1), pltpu.roll(zi, 2, 1))
        wa, wb = _dot(jnp.where(own, zr, zi), fd[2]), _dot(jnp.where(own, zi, zr), fd[3])
        total, diff = wa + wb, wa - wb
        other = pltpu.roll(diff, 64, 1)
        v0 = jnp.where(lo, total, (other + diff) * _R2)
        v1 = jnp.where(lo, pltpu.roll(total, 64, 1), (diff - other) * _R2)
        e0, e1 = u0 + u2, u0 - u2
        for j, y in enumerate((e0 + v0, e1 + v1, e0 - v0, e1 - v1)):
            y = y * (2.0 / (S * D))
            y = pltpu.bitcast(y.astype(BF16).astype(F32), U32)
            y = _pack(y[:128], y[128:])
            for sigma in range(2):
                ya[c, j, pl.ds(sigma, 64, stride=2), :] = y[64 * sigma:64 * (sigma + 1)]

    part = {}

    def combine(spec, block):
        a, b = block(*spec[0]), block(*spec[1])
        return (a + b if spec[2] > 0 else a - b).astype(BF16)

    def early(p, n, mc):
        _, right, uses = _PRODUCTS[n]
        x = xs[n, (pinned if isinstance(p, int) else rows)(0, 64 * mc, 64), :]
        if mc == 1:
            x = jnp.concatenate([after_stores(x[:, :128]), x[:, 128:]], axis=1)
        elif len(right) > 1:
            def block(r, c):
                words = raw[p, pl.ds(D // 2 * r, D // 2), :]
                return (_lo, _hi)[c](after_stores(words) if (r, c) == right[0] else words)

            part["w"] = combine(right, block)
        else:
            r, c = right[0]
            even, odd = [raw[p, pl.ds(D // 2 * r + t, D // 4, stride=2), :] for t in range(2)]
            plain = (even & np.uint32(0xFFFF)) | (odd << 16), _pack(even, odd)
            part["w"] = pltpu.bitcast(after_stores(plain[c]), BF16)
            for h in range(2):
                work[rows(p * D, h * (D // 2) + r * (D // 4), D // 4), :] = plain[h]
        prod = _dot(pltpu.bitcast(x, BF16), part["w"])
        for key, sign in uses:
            total, count = part.pop((key, mc), (None, 0))
            total = prod if total is None else (total + prod if sign > 0 else total - prod)
            if count + 1 == (4 if key[0] == key[1] else 2):
                pre[rows(p * 16 * NSEG, key[1] * 8 * NSEG + 4 * NSEG * key[0] + 128 * mc, 128), :] = total
            else:
                part[key, mc] = total, count + 1

    def early_work(phase, i):
        first, count, _ = PHASES[phase]
        wait_for(raw.at[pl.ds(first + count * i, count), pl.ds(0, D)], sem_phase[phase] + i)
        return [(early, (first + count * i + u, n, mc)) for u in range(count) for n in range(7) for mc in range(2)]

    def run(order, **queues):
        for name in order:
            fn, args = queues[name].pop(0)
            fn(*args)
        assert not any(queues.values())

    def plain_phase(phase, i):
        todo = early_work(phase, i)
        run("P" * len(todo), P=todo)

    def forward_phase(i):
        wait_for(ax.at[i], sem_x + i)
        wait_for(gt.at[i], sem_g + i)
        run(ORDER_FORWARD, P=early_work(2, i),
            O=[(a_features, (i, u, n)) for u in range(4) for n in range(4)],
            T=[(a_time, (i, u, half, sigma)) for u in range(4) for half in range(2) for sigma in range(2)],
            S=[(a_spread, (i, half, jg)) for jg in range(9) for half in range(2)])

    def filter_phase(i):
        run(ORDER_FILTER, P=early_work(3, i), F=[w for jg in range(4) for blk in range(4) for w in filter_work(i, jg, blk)])

    wait(0)
    xp = xpre[...].reshape(8 * NSEG, D)

    def block_of_x(r, c):
        return xp[256 * r:256 * (r + 1), 256 * c:256 * (c + 1)]

    for n, (left, _, _) in enumerate(_PRODUCTS):
        x = block_of_x(*left[0]) if len(left) == 1 else combine(left, lambda r, c: block_of_x(r, c).astype(F32))
        xs[n] = pltpu.bitcast(x, U32)
    plain_phase(0, 0)
    pl.loop(0, PHASES[1][2])(lambda i: plain_phase(1, i))
    wait(sem_fd)
    pl.loop(0, 2)(forward_phase)
    wait(sem_filter)
    run("F" * 6, F=filter_work(0, 0, 4))
    pl.loop(0, 2)(filter_phase)
    wait(sem_rest)

    row = lax.broadcasted_iota(jnp.int32, (L, L), 0)
    col = lax.broadcasted_iota(jnp.int32, (L, L), 1)
    mask = (row >= SEG) | (col >= SEG) | (row >= col)
    scale = DH ** -0.5

    def w_in(i, g):
        return jnp.concatenate(
            [pltpu.bitcast(work[pl.ds((i * H + 4 * g + j) * (D // 2), D // 2), :], BF16) for j in range(4)], axis=1)

    def w_out(g):
        return jnp.concatenate([pltpu.bitcast(wo[j, 256 * g:256 * (g + 1)], BF16) for j in range(4)], axis=1)

    def step(s, carry, c=None):
        mem, late_o, late_acc = carry
        h = jnp.concatenate([xrest[s].astype(F32), mem], axis=0).astype(BF16)
        st = {"late": late_acc}

        def project(i, g):
            known = [pre[pl.ds(pl.multiple_of(s * 8, 8) + (i * H + 4 * g + j) * 8 * NSEG, 8), :] for j in range(4)]
            st[i, g] = jnp.concatenate([jnp.concatenate(known, axis=1), _dot(h, w_in(i, g))], axis=0)

        def softmax(g):
            ps = []
            for j in range(4):
                cols = slice(DH * j, DH * (j + 1))
                sc = _dot(st[0, g][:, cols], st[1, g][:, cols], NT)
                sc = jnp.where(mask, sc * (scale * LOG2E), -1e9 * LOG2E)
                e = jnp.exp2(sc - jnp.max(sc, axis=1, keepdims=True))
                total = jnp.sum(e, axis=1, keepdims=True)
                r = pltpu.reciprocal(total, approx=True)
                ps.append((e, r * (2.0 - total * r)))
            st["p", g] = ps

        def mix_rows(g, which):
            v = st[2, g].astype(BF16)
            return jnp.concatenate([_dot(e[which], v[:, DH * j:DH * (j + 1)]) * r[which]
                                    for j, (e, r) in enumerate(st["p", g])], axis=1)

        def mix(g):
            if g >= 8 - LATE:
                st["o", g] = jnp.concatenate([mix_rows(g, slice(SEG, L)), late_o[g - (8 - LATE)]], axis=0)
            else:
                o = mix_rows(g, slice(0, L))
                st["o", g] = jnp.concatenate([o[SEG:], o[:SEG]], axis=0)

        def output(g):
            r = _dot(st["o", g], w_out(g))
            st["mem"] = r[:M] if g == 0 else st["mem"] + r[:M]
            key = "late" if g >= 8 - LATE else "tokens"
            st[key] = r[M:] if g == 0 else st[key] + r[M:]

        for g in range(8):
            project(1, g)
            project(0, g)
            if g > 0:
                mix(g - 1)
            project(2, g)
            softmax(g)
        if c is not None:
            z = a_inverse_time(c)
        for g in range(8):
            output(g)
            if g == 1:
                mix(7)
            if g == 3 and c is not None:
                a_inverse_features(c, *z)
        late_o = tuple(mix_rows(g, slice(0, SEG)) for g in range(8 - LATE, 8))
        yb[pl.ds(2 * s, 2)] = st["late"].astype(BF16).reshape(2, 16, D)
        return st["mem"], late_o, st["tokens"]

    def b_out(first, n):
        return pltpu.make_async_copy(
            yb.at[pl.ds(2 * first + 2, 2 * n)], out_hbm.at[pl.ds(2 * first, 2 * n), :, pl.ds(D, D)], sems.at[sem_b])

    def block(i, carry):
        for u in range(STEPS):
            carry = step(i * STEPS + u, carry, i if u == STEPS - 1 else None)
        for j in range(4):
            pltpu.make_async_copy(
                ya.at[i, j, pl.ds(0, 128)], out32.at[:, i, pl.ds(128 * j, 128)], sems.at[sem_a]).start()

        @pl.when(i == 0)
        def _():
            b_out(0, STEPS - 1).start()

        @pl.when(i > 0)
        def _():
            b_out(i * STEPS - 1, STEPS).start()

        return carry

    zeros = jnp.zeros((SEG, D), F32)
    _, late_o, acc = lax.fori_loop(0, NSEG // STEPS, block, (mem0[...].astype(F32), (zeros,) * LATE, zeros))
    for g in range(8 - LATE, 8):
        acc = acc + _dot(late_o[g - (8 - LATE)], w_out(g))
    yb[pl.ds(2 * NSEG, 2)] = acc.astype(BF16).reshape(2, 16, D)
    b_out(NSEG - 1, 1).start()
    wait_for(ya.at[:, :, pl.ds(0, 128)], sem_a)
    b_out(0, NSEG).wait()


def _forward(A_x, A_w_r, A_w_i, B_x, B_mem0, B_Wq, B_Wk, B_Wv, B_Wo):
    in_hbm = pl.BlockSpec(memory_space=pl.ANY)
    out = pl.pallas_call(
        _kernel,
        out_shape=jax.ShapeDtypeStruct((S // 16, 16, 2 * D), BF16),
        in_specs=[in_hbm] * 13,
        out_specs=in_hbm,
        scratch_shapes=[
            pltpu.VMEM((2, 4, 2, 64, D), U32),
            pltpu.VMEM((D // 4, S), U32),
            pltpu.VMEM((D // 4, S), U32),
            pltpu.VMEM((1, S), BF16),
            pltpu.VMEM((1, S), BF16),
            pltpu.VMEM((5, 128, 128), BF16),
            pltpu.VMEM((2, 4, 2, 2, 128, 128), BF16),
            pltpu.VMEM((16, 8, 128), F32),
            pltpu.VMEM((NYQ + 256, 128), F32),
            pltpu.VMEM((ZERO + 8, 128), U32),
            pltpu.VMEM((8, 4, 128 + 32, 128), U32),
            pltpu.VMEM((PAIRS, D + 32, 128), U32),
            pltpu.VMEM((7, 2 * NSEG, D // 2), U32),
            pltpu.VMEM((4, H * DH // 2, 128), U32),
            pltpu.VMEM((NSEG, 8, D), BF16),
            pltpu.VMEM((NSEG, SEG - 8, D), BF16),
            pltpu.VMEM((M, D), BF16),
            pltpu.VMEM((3 * H * 8 * NSEG, DH), F32),
            pltpu.VMEM((2 * NSEG + 2, 16, D), BF16),
            pltpu.SMEM((128,), jnp.int32),
            pltpu.SemaphoreType.DMA((10 + sum(p[2] for p in PHASES),)),
        ],
        compiler_params=pltpu.CompilerParams(vmem_limit_bytes=100 * 1024 * 1024),
    )(A_x.reshape(S // 32, 32, D), A_w_r.T, A_w_i.T, B_x.reshape(NSEG, SEG, D), B_mem0.reshape(M, D),
      B_Wq, B_Wk, B_Wv, B_Wo.reshape(H * DH, D), _FD, _G, _TURNS, _INDICES)
    return out.reshape(1, S, 2 * D)


@jax.jit
def pallas_concat_heads__spectral_gfnet__memory_aug_recurrent_mem_tr__prompt_kernel(
    A_x: jax.Array,
    A_w_r: jax.Array,
    A_w_i: jax.Array,
    B_x: jax.Array,
    B_mem0: jax.Array,
    B_Wq: jax.Array,
    B_Wk: jax.Array,
    B_Wv: jax.Array,
    B_Wo: jax.Array,
    B_seg_len: jax.Array,
):
    del B_seg_len
    return _forward(A_x, A_w_r, A_w_i, B_x, B_mem0, B_Wq, B_Wk, B_Wv, B_Wo)
```

```python
import jax
import jax.numpy as jnp
import numpy as np
from jax import lax
import jax.experimental.pallas as pl
import jax.experimental.pallas.tpu as pltpu

F32, BF16, U32 = jnp.float32, jnp.bfloat16, jnp.uint32
NN = (((1,), (0,)), ((), ()))
NT = (((1,), (1,)), ((), ()))

S, D = 2048, 512
M, SEG, H, DH = 8, 32, 32, 128
L = M + SEG
NSEG = S // SEG
LOG2E = 1.4426950408889634

STEPS = 8
LATE = 3
PAIRS = 3 * H // 2
PHASES = ((0, 2, 1), (2, 4, 3), (14, 5, 2), (24, 12, 2))
ORDER_FORWARD = ("PPOOPOOOTTOOTOTPTOOTOOOTTPTTTTOOPOPPTTPPPPTTPPPPPPPPSPPPSPSPSPPSPPSPPPPPPSPSPSPPSPPSPPPSPPSPPSPPPPSPSPPP"
                 "SPSPPPPPPPPPPPPP")
ORDER_FILTER = 2 * ("PPFPFPFPFPPFPPFPPFPPFPFPPFPPFPFPPFPPFPPFPPFPPPFPFPFPFPPFPPFPPFPPFPPFPFPPFPFPPPFPFPPFPPFPFPPFPPFP"
                    "FPPFPPFPPFPPFPPFPPFPFPFPPPFPFPPFPPFP")
SPEC = 3 * H * D // 2
NYQ = 16 * 512
ZERO = SPEC + NYQ + 256


def _dft_constants():
    d = np.arange(128)
    j = (8 * np.arange(8)[:, None] + np.array([0, 4, 1, 5, 2, 6, 3, 7])[None, :]).reshape(-1)

    def cos_sin(r):
        ang = 2 * np.pi * (np.outer(4 * j + r, d) % D) / D
        return np.cos(ang), np.sin(ang)

    (c0, s0), (c1, s1), (c2, s2), (c3, s3) = [cos_sin(r) for r in range(4)]
    f0 = np.concatenate([c0, -s0])
    f0[64] = 1.0 - 2.0 * (d % 2)
    row = np.arange(128)
    cos, sin = np.concatenate([c1, c3])[:, :64], np.concatenate([s1, s3])[:, :64]
    sign = np.where(row < 64, -1.0, 1.0)[:, None]
    real, imag = np.concatenate([cos, sign * sin], axis=1), np.concatenate([-sin, sign * cos], axis=1)[row ^ 2]
    own = (((row & 2) == 0) == (row < 64))[:, None]
    fd = np.stack([f0, np.concatenate([c2, -s2]), np.where(own, real, imag), np.where(own, imag, real),
                   np.concatenate([-s2, c2])])
    i, u, half, sigma, t1, f1 = np.ix_(*[np.arange(n) for n in (2, 4, 2, 2, 64, 64)])
    ang = 2 * np.pi * (((32 * t1 + 16 * sigma + 4 * u + 2 * i + half) * f1) % S) / S
    gr, gi = np.cos(ang), -np.sin(ang)
    g = np.concatenate([np.concatenate([gr, gi], axis=-1), np.concatenate([-gi, gr], axis=-1)], axis=-2)
    ang = 2 * np.pi * np.arange(16)[:, None, None] / 32
    low = np.arange(128)[None, None, :] < 64
    turns = np.concatenate([np.cos(ang) * np.ones_like(low), np.where(low, -np.sin(ang), np.sin(ang)),
                            np.zeros((16, 6, 128))], axis=1)

    def words(a):
        bits = a.astype(np.float32).astype(BF16).view(np.uint16).astype(np.uint32).reshape(-1, 128)
        return bits[0::2] | (bits[1::2] << 16)

    return words(fd), words(g), turns.astype(np.float32)


_FD, _G, _TURNS = _dft_constants()
_INDICES = np.arange(128, dtype=np.int32) ** 2
_C8, _S8, _R2 = float(np.cos(np.pi / 8)), float(np.sin(np.pi / 8)), float(np.sqrt(0.5))

_PRODUCTS = (
    (((0, 0), (1, 1), 1), ((0, 0), (1, 1), 1), (((0, 0), 1), ((1, 1), 1))),
    (((1, 0), (1, 1), 1), ((0, 0),), (((1, 0), 1), ((1, 1), -1))),
    (((1, 1),), ((1, 0), (0, 0), -1), (((0, 0), 1), ((1, 0), 1))),
    (((0, 0), (0, 1), 1), ((1, 1),), (((0, 0), -1), ((0, 1), 1))),
    (((0, 1), (1, 1), -1), ((1, 0), (1, 1), 1), (((0, 0), 1),)),
    (((0, 0),), ((0, 1), (1, 1), -1), (((0, 1), 1), ((1, 1), 1))),
    (((1, 0), (0, 0), -1), ((0, 0), (0, 1), 1), (((1, 1), 1),)),
)


def _dot(a, b, dims=NN):
    return lax.dot_general(a, b, dims, preferred_element_type=F32)


def _radix4(a, b, c, d, sign):
    t0 = (a[0] + c[0], a[1] + c[1])
    t1 = (a[0] - c[0], a[1] - c[1])
    t2 = (b[0] + d[0], b[1] + d[1])
    t3 = (b[0] - d[0], b[1] - d[1])
    y0 = (t0[0] + t2[0], t0[1] + t2[1])
    y2 = (t0[0] - t2[0], t0[1] - t2[1])
    ya = (t1[0] + t3[1], t1[1] - t3[0])
    yb = (t1[0] - t3[1], t1[1] + t3[0])
    return (y0, ya, y2, yb) if sign < 0 else (y0, yb, y2, ya)


def _twiddle16(z, e):
    re, im = z
    if e == 0:
        return z
    if e == 4:
        return -im, re
    if e == 2:
        return (re - im) * _R2, (im + re) * _R2
    if e == 6:
        return (re + im) * (-_R2), (re - im) * _R2
    c, s = {1: (_C8, _S8), 3: (_S8, _C8), 9: (-_C8, -_S8)}[e]
    return re * c - im * s, im * c + re * s


def _lo(w):
    return pltpu.bitcast(w << 16, F32)


def _hi(w):
    return pltpu.bitcast(w & np.uint32(0xFFFF0000), F32)


def _pack(even, odd):
    return (even >> 16) | (odd & np.uint32(0xFFFF0000))


def _kernel(ax_hbm, wr_hbm, wi_hbm, bx_hbm, mem_hbm, wq_hbm, wk_hbm, wv_hbm, wo_hbm, fd_hbm, g_hbm, turns_hbm,
            idx_hbm, out_hbm,
            turns, ax, wr, wi, fd, gt, ybuf, work, ya, raw, xs, wo, xpre, xrest, pre, yb, mem0, wr_last, wi_last, idx,
            sems):
    ax32 = ax_hbm.bitcast(U32)
    wo32 = wo_hbm.bitcast(U32)
    out32 = out_hbm.bitcast(U32)
    w32 = [w.bitcast(U32) for w in (wq_hbm, wk_hbm, wv_hbm)]

    sem_phase = [1 + sum(p[2] for p in PHASES[:n]) for n in range(5)]
    sem_fd, sem_filter, sem_rest, sem_a, sem_b, sem_x, sem_g = [sem_phase[4] + n for n in (0, 1, 2, 3, 4, 5, 7)]

    def pairs(phase, i):
        first, count, _ = PHASES[phase]
        return [(w32[p // 16].at[:, p % 16, :], raw.at[p, pl.ds(0, D)], sem_phase[phase] + i)
                for p in range(first + count * i, first + count * (i + 1))]

    def filters(src, dst, last):
        return [(src.at[pl.ds(0, D // 2)].bitcast(U32), dst, sem_filter), (src.at[pl.ds(D // 2, 1)], last, sem_filter)]

    plan = [(idx_hbm, idx, 0), (bx_hbm.at[:, pl.ds(0, 8), :], xpre, 0)] + pairs(0, 0)
    for i in range(PHASES[1][2]):
        plan += pairs(1, i)
    plan += [(fd_hbm, fd, sem_fd)]
    for i in range(2):
        plan += pairs(2, i)
        plan += [(ax32.at[:, 8 * sigma + 2 * u + i, :], ax.at[i, u, sigma], sem_x + i)
                 for u in range(4) for sigma in range(2)]
        plan += [(g_hbm.at[pl.ds(1024 * i, 1024)], gt.at[pl.ds(1024 * i, 1024)], sem_g + i)]
    plan += filters(wr_hbm, wr, wr_last) + filters(wi_hbm, wi, wi_last)
    for i in range(PHASES[3][2]):
        plan += pairs(3, i)
    plan += [(turns_hbm, turns, sem_rest), (mem_hbm, mem0, sem_rest),
             (bx_hbm.at[:, pl.ds(8, SEG - 8), :], xrest, sem_rest)]
    plan += [(wo32.at[:, pl.ds(128 * j, 128)], wo.at[j], sem_rest) for j in range(4)]
    for src, dst, sem in plan:
        pltpu.make_async_copy(src, dst, sems.at[sem]).start()

    def wait(sem):
        for src, dst, n in plan:
            if n == sem:
                pltpu.make_async_copy(src, dst, sems.at[sem]).wait()

    def wait_for(dst, sem):
        pltpu.make_async_copy(dst, dst, sems.at[sem]).wait()

    sub = lax.broadcasted_iota(jnp.int32, (8, 128), 0)
    lane = lax.broadcasted_iota(jnp.int32, (264, 128), 1)
    low = lane < 64
    row0 = sub == 0

    def rows(base, off, n, stride=1):
        return pl.ds((base if isinstance(base, int) else pl.multiple_of(base, 32)) + off, n, stride)

    def pinned(base, off, n):
        return rows(idx[0] + base, off, n)

    work[pl.ds(ZERO, 8), :] = jnp.zeros((8, 128), U32)

    def after_stores(words):
        return jnp.concatenate([words[:8] | work[pinned(ZERO, 0, 8), :], words[8:]], axis=0)

    def get(where):
        return pltpu.bitcast(work[where, :], F32)

    def put(where, v):
        work[where, :] = pltpu.bitcast(v, U32)

    fw = {}

    def table(n):
        return pltpu.bitcast(fd[pl.ds(64 * n, 64), :], BF16)

    def by_group(v):
        return jnp.concatenate([v[64 * blk + 8 * jg:64 * blk + 8 * jg + 8] for jg in range(8) for blk in range(4)], 0)

    def by_block(v):
        return jnp.concatenate([v[32 * jg + 8 * blk:32 * jg + 8 * blk + 8] for blk in range(4) for jg in range(8)], 0)

    def a_features(i, u, n):
        if n == 0:
            words = [jnp.concatenate([ax[i, u, sigma, :, 128 * j:128 * (j + 1)] for sigma in range(2)], axis=0)
                     for j in range(4)]
            x = [jnp.concatenate([_lo(w), _hi(w)], axis=0) for w in words]
            a0, a1, b0, b1 = x[0] + x[2], x[1] + x[3], x[0] - x[2], x[1] - x[3]
            base = jnp.where(low[:256], b0, pltpu.roll(b1, 64, 1))
            t = jnp.where(low[:256], pltpu.roll(b0 - b1, 64, 1), b0 + b1) * _R2
            fw[u] = [v.astype(BF16) for v in (a0 + a1, a0 - a1, base + t, base - t)]
        fw[u][n] = _dot(table(n), fw[u][n], NT)

    def a_time(i, u, half, sigma):
        if half == 0 and sigma == 0:
            e0, e2, qa, qb = fw[u]
            first = jnp.concatenate([(sub & 2) == 0] * 2, axis=1)
            re, im = [], []
            for r in range(0, 128, 8):
                x, y = (qa[r:r + 8], qb[r:r + 8]) if r < 64 else (qb[r:r + 8], qa[r:r + 8])
                re.append(jnp.where(first, x, y))
                t = jnp.where(first, y, x)
                im.append(jnp.where(first, pltpu.roll(t, 6, 0), pltpu.roll(t, 2, 0)))
            nyq = e0[64:72]
            fw[u] = (jnp.concatenate([e0[:64], e2[:64]] + re + [nyq], axis=0),
                     jnp.concatenate([jnp.where(jnp.concatenate([row0, row0], axis=1), 0.0, nyq), e0[72:], e2[64:]]
                                     + im + [jnp.zeros_like(nyq)], axis=0))
        g = pltpu.bitcast(gt[rows(1024 * i, 256 * u + 128 * half + 64 * sigma, 64), :], BF16)
        if sigma == 0:
            xr, xi = [v[:, 128 * half:128 * (half + 1)] for v in fw[u]]
            xi = pltpu.roll(xi, 64, 1)
            fw["odd"] = jnp.where(low, xi, xr)
            fw["even"] = _dot(jnp.where(low, xr, xi), g)
            return
        odd = _dot(fw["odd"], jnp.concatenate([g[64:], g[:64]], axis=0))
        total, diff = fw["even"] + odd, fw["even"] - odd
        c, s = [jnp.where(i == 0, f(2 * np.pi * (4 * u + half) / 32), f(2 * np.pi * (4 * u + half + 2) / 32)).astype(F32)
                for f in (np.cos, np.sin)]
        other = pltpu.roll(diff, 64, 1)
        for d, y in enumerate((jnp.where(low, total, c * other + s * diff),
                               jnp.where(low, pltpu.roll(total, 64, 1), c * diff - s * other))):
            ybuf[rows(1024 * i, 2048 * u + 512 * half + 256 * d, 256), :] = by_group(y[:256])
            ybuf[rows(32 * i, NYQ + 64 * u + 16 * half + 8 * d, 8), :] = y[256:]

    def a_spread(i, half, jg):
        tw = [[jnp.where(i == 0, f(2 * np.pi * half * k / 16), f(2 * np.pi * (2 + half) * k / 16)).astype(F32)
               for f in (np.cos, np.sin)] for k in range(4)]
        if jg == 8:
            todo = [[(32 * i, NYQ + 64 * u + 16 * half, 8) for u in range(4)]]
        else:
            todo = [[(1024 * i, 2048 * u + 512 * half + 32 * jg + 8 * blk, 256) for u in range(4)] for blk in range(4)]
        for slots in todo:
            x = _radix4(*[(ybuf[pinned(b, o, 8), :], ybuf[pinned(b, o + d, 8), :]) for b, o, d in slots], -1)
            for k, ((b, o, d), (re, im)) in enumerate(zip(slots, x)):
                if k > 0:
                    c, s = tw[k]
                    re, im = re * c + im * s, im * c - re * s
                put(rows(b, SPEC + o, 8), re)
                put(rows(b, SPEC + o + d, 8), im)

    def weight(i, jg, blk, f):
        cols = slice(128 * f, 128 * (f + 1))
        if blk == 4:
            return tuple(jnp.broadcast_to(r[:, cols].astype(F32) * 0.5, (8, 128)) for r in (wr_last, wi_last))
        out = []
        for r in (wr, wi):
            v = r[rows(64 * i, 16 * jg, 16), cols]
            if blk % 2 == 0:
                v = jnp.where(sub % 2 == 0, v[:8], pltpu.roll(v[8:], 1, 0))
            else:
                v = jnp.where(sub % 2 == 0, pltpu.roll(v[:8], 7, 0), v[8:])
            v = _lo(v) if blk < 2 else _hi(v)
            if blk == 0 and jg == 0:
                v = v * jnp.where(jnp.logical_and(row0, i == 0), 0.5, 1.0).astype(F32)
            out.append(v)
        return tuple(out)

    def slot(jg, blk, s):
        if blk == 4:
            return SPEC + NYQ + 16 * s, SPEC + NYQ + 16 * s + 8
        return SPEC + 512 * s + 32 * jg + 8 * blk, SPEC + 512 * s + 256 + 32 * jg + 8 * blk

    def a_filter(i, jg, blk, t):
        slots = [slot(jg, blk, 4 * t + u) for u in range(4)]
        x = _radix4(*[tuple(get(pinned(128 * i, r, 8)) for r in ri) for ri in slots], -1)
        w = [weight(i, jg, blk, t + 4 * k) for k in range(4)]
        x = [(v[0] * u[0] - v[1] * u[1], v[0] * u[1] + v[1] * u[0]) for v, u in zip(x, w)]
        for n, (ri, v) in enumerate(zip(slots, _radix4(*x, +1))):
            v = _twiddle16(v, t * n)
            put(rows(128 * i, ri[0], 8), v[0])
            put(rows(128 * i, ri[1], 8), v[1])

    def a_gather(i, jg, blk, ts):
        todo = [[slot(jg, blk, 4 * u + t) for u in range(4)] for t in ts]
        values = [[tuple(get(pinned(128 * i, r, 8)) for r in ri) for ri in slots] for slots in todo]
        for slots, x in zip(todo, values):
            for ri, v in zip(slots, _radix4(*x, +1)):
                put(rows(128 * i, ri[0], 8), v[0])
                put(rows(128 * i, ri[1], 8), v[1])

    def filter_work(i, jg, blk):
        return [(a_filter, (i, jg, blk, t)) for t in range(4)] + [(a_gather, (i, jg, blk, ts)) for ts in ((0, 1), (2, 3))]

    def a_inverse_time(c):
        zr, zi = [], []
        for half in range(2):
            ur, ui = [jnp.concatenate([by_block(get(rows(1024 * c, SPEC + 512 * half + 256 * d, 256))),
                                       get(rows(32 * c, SPEC + NYQ + 16 * half + 8 * d, 8))], axis=0)
                      for d in range(2)]
            co, si = turns[2 * c + half, 0:1], turns[2 * c + half, 1:2]
            moved = pltpu.roll(ui, 64, 1)
            base = jnp.where(low, ur, moved)
            t = co * jnp.where(low, pltpu.roll(ur, 64, 1), ui) + si * jnp.where(low, moved, ur)
            for sigma, v in enumerate((base + t, base - t)):
                g = pltpu.bitcast(gt[rows(1024 * (c % 2) + 256 * (c // 2), 128 * half + 64 * sigma, 64), :], BF16)
                k = _dot(g, v[:256].astype(BF16), NT)
                nyq = jnp.sum(g[:64].astype(F32) * v[256:257], axis=1, keepdims=True)
                zr.append(k[:64])
                zi.append(jnp.concatenate([jnp.where(lane[:64] == 0, nyq, k[64:, :128]), k[64:, 128:]], axis=1))
        return jnp.concatenate(zr, axis=0), jnp.concatenate(zi, axis=0)

    def a_inverse_features(c, zr, zi):
        lo = low[:256]
        rot = pltpu.roll(zi[:, :128], 64, 1)
        u0 = _dot(jnp.where(lo, zr[:, :128], rot), table(0))
        u2 = _dot(jnp.where(lo, rot, zr[:, :128]), table(4))
        zr, zi = zr[:, 128:], zi[:, 128:]
        first = (lane[:256] & 2) == 0
        own = first == lo
        zi = jnp.where(first, pltpu.roll(zi, 126, 1), pltpu.roll(zi, 2, 1))
        wa, wb = _dot(jnp.where(own, zr, zi), table(2)), _dot(jnp.where(own, zi, zr), table(3))
        total, diff = wa + wb, wa - wb
        other = pltpu.roll(diff, 64, 1)
        v0 = jnp.where(lo, total, (other + diff) * _R2)
        v1 = jnp.where(lo, pltpu.roll(total, 64, 1), (diff - other) * _R2)
        e0, e1 = u0 + u2, u0 - u2
        for j, y in enumerate((e0 + v0, e1 + v1, e0 - v0, e1 - v1)):
            y = y * (2.0 / (S * D))
            y = pltpu.bitcast(y.astype(BF16).astype(F32), U32)
            y = _pack(y[:128], y[128:])
            for sigma in range(2):
                ya[pl.ds(pl.multiple_of(512 * c, 32) + 128 * j + sigma, 64, stride=2), :] = y[64 * sigma:64 * (sigma + 1)]

    part = {}

    def combine(spec, block):
        a, b = block(*spec[0]), block(*spec[1])
        return (a + b if spec[2] > 0 else a - b).astype(BF16)

    def early(p, n, mc):
        _, right, uses = _PRODUCTS[n]
        x = xs[n, (pinned if isinstance(p, int) else rows)(0, 64 * mc, 64), :]
        if mc == 1:
            x = jnp.concatenate([after_stores(x[:, :128]), x[:, 128:]], axis=1)
        elif len(right) > 1:
            def block(r, c):
                words = raw[p, pl.ds(D // 2 * r, D // 2), :]
                return (_lo, _hi)[c](after_stores(words) if (r, c) == right[0] else words)

            part["w"] = combine(right, block)
        else:
            r, c = right[0]
            even, odd = [raw[p, pl.ds(D // 2 * r + t, D // 4, stride=2), :] for t in range(2)]
            plain = (even & np.uint32(0xFFFF)) | (odd << 16), _pack(even, odd)
            part["w"] = pltpu.bitcast(after_stores(plain[c]), BF16)
            for h in range(2):
                work[rows(p * D, h * (D // 2) + r * (D // 4), D // 4), :] = plain[h]
        prod = _dot(pltpu.bitcast(x, BF16), part["w"])
        for key, sign in uses:
            total, count = part.pop((key, mc), (None, 0))
            total = prod if total is None else (total + prod if sign > 0 else total - prod)
            if count + 1 == (4 if key[0] == key[1] else 2):
                pre[rows(p * 16 * NSEG, key[1] * 8 * NSEG + 4 * NSEG * key[0] + 128 * mc, 128), :] = total
            else:
                part[key, mc] = total, count + 1

    def early_work(phase, i):
        first, count, _ = PHASES[phase]
        wait_for(raw.at[pl.ds(first + count * i, count), pl.ds(0, D)], sem_phase[phase] + i)
        return [(early, (first + count * i + u, n, mc)) for u in range(count) for n in range(7) for mc in range(2)]

    def run(order, **queues):
        for name in order:
            fn, args = queues[name].pop(0)
            fn(*args)
        assert not any(queues.values())

    def plain_phase(phase, i):
        todo = early_work(phase, i)
        run("P" * len(todo), P=todo)

    def forward_phase(i):
        wait_for(ax.at[i], sem_x + i)
        wait_for(gt.at[rows(1024 * i, 0, 1024)], sem_g + i)
        run(ORDER_FORWARD, P=early_work(2, i),
            O=[(a_features, (i, u, n)) for u in range(4) for n in range(4)],
            T=[(a_time, (i, u, half, sigma)) for u in range(4) for half in range(2) for sigma in range(2)],
            S=[(a_spread, (i, half, jg)) for jg in range(9) for half in range(2)])

    def filter_phase(i):
        run(ORDER_FILTER, P=early_work(3, i), F=[w for jg in range(4) for blk in range(4) for w in filter_work(i, jg, blk)])

    wait(0)
    xp = xpre[...].reshape(8 * NSEG, D)

    def block_of_x(r, c):
        return xp[256 * r:256 * (r + 1), 256 * c:256 * (c + 1)]

    for n, (left, _, _) in enumerate(_PRODUCTS):
        x = block_of_x(*left[0]) if len(left) == 1 else combine(left, lambda r, c: block_of_x(r, c).astype(F32))
        xs[n] = pltpu.bitcast(x, U32)
    plain_phase(0, 0)
    pl.loop(0, PHASES[1][2])(lambda i: plain_phase(1, i))
    wait(sem_fd)
    pl.loop(0, 2)(forward_phase)
    wait(sem_filter)
    run("F" * 6, F=filter_work(0, 0, 4))
    pl.loop(0, 2)(filter_phase)
    wait(sem_rest)

    row = lax.broadcasted_iota(jnp.int32, (L, L), 0)
    col = lax.broadcasted_iota(jnp.int32, (L, L), 1)
    mask = (row >= SEG) | (col >= SEG) | (row >= col)
    scale = DH ** -0.5

    def w_in(i, g):
        return jnp.concatenate(
            [pltpu.bitcast(work[pl.ds((i * H + 4 * g + j) * (D // 2), D // 2), :], BF16) for j in range(4)], axis=1)

    def w_out(g):
        return jnp.concatenate([pltpu.bitcast(wo[j, 256 * g:256 * (g + 1)], BF16) for j in range(4)], axis=1)

    def step(s, carry, c=None):
        mem, late_o, late_acc = carry
        h = jnp.concatenate([xrest[s].astype(F32), mem], axis=0).astype(BF16)
        st = {"late": late_acc}

        def project(i, g):
            known = [pre[pl.ds(pl.multiple_of(s * 8, 8) + (i * H + 4 * g + j) * 8 * NSEG, 8), :] for j in range(4)]
            st[i, g] = jnp.concatenate([jnp.concatenate(known, axis=1), _dot(h, w_in(i, g))], axis=0)

        def softmax(g):
            ps = []
            for j in range(4):
                cols = slice(DH * j, DH * (j + 1))
                sc = _dot(st[0, g][:, cols], st[1, g][:, cols], NT)
                sc = jnp.where(mask, sc * (scale * LOG2E), -1e9 * LOG2E)
                e = jnp.exp2(sc - jnp.max(sc, axis=1, keepdims=True))
                total = jnp.sum(e, axis=1, keepdims=True)
                r = pltpu.reciprocal(total, approx=True)
                ps.append((e, r * (2.0 - total * r)))
            st["p", g] = ps

        def mix_rows(g, which):
            v = st[2, g].astype(BF16)
            return jnp.concatenate([_dot(e[which], v[:, DH * j:DH * (j + 1)]) * r[which]
                                    for j, (e, r) in enumerate(st["p", g])], axis=1)

        def mix(g):
            if g >= 8 - LATE:
                st["o", g] = jnp.concatenate([mix_rows(g, slice(SEG, L)), late_o[g - (8 - LATE)]], axis=0)
            else:
                o = mix_rows(g, slice(0, L))
                st["o", g] = jnp.concatenate([o[SEG:], o[:SEG]], axis=0)

        def output(g):
            r = _dot(st["o", g], w_out(g))
            st["mem"] = r[:M] if g == 0 else st["mem"] + r[:M]
            key = "late" if g >= 8 - LATE else "tokens"
            st[key] = r[M:] if g == 0 else st[key] + r[M:]

        for g in range(8):
            project(1, g)
            project(0, g)
            if g > 0:
                mix(g - 1)
            project(2, g)
            softmax(g)
        if c is not None:
            z = a_inverse_time(c)
        for g in range(8):
            output(g)
            if g == 1:
                mix(7)
            if g == 3 and c is not None:
                a_inverse_features(c, *z)
        late_o = tuple(mix_rows(g, slice(0, SEG)) for g in range(8 - LATE, 8))
        yb[pl.ds(2 * s, 2)] = st["late"].astype(BF16).reshape(2, 16, D)
        return st["mem"], late_o, st["tokens"]

    def b_out(first, n):
        return pltpu.make_async_copy(
            yb.at[pl.ds(2 * first + 2, 2 * n)], out_hbm.at[pl.ds(2 * first, 2 * n), :, pl.ds(D, D)], sems.at[sem_b])

    def block(i, carry):
        for u in range(STEPS):
            carry = step(i * STEPS + u, carry, i if u == STEPS - 1 else None)
        for j in range(4):
            pltpu.make_async_copy(
                ya.at[rows(512 * i, 128 * j, 128)], out32.at[:, i, pl.ds(128 * j, 128)], sems.at[sem_a]).start()

        @pl.when(i == 0)
        def _():
            b_out(0, STEPS - 1).start()

        @pl.when(i > 0)
        def _():
            b_out(i * STEPS - 1, STEPS).start()

        return carry

    zeros = jnp.zeros((SEG, D), F32)
    _, late_o, acc = lax.fori_loop(0, NSEG // STEPS, block, (mem0[...].astype(F32), (zeros,) * LATE, zeros))
    for g in range(8 - LATE, 8):
        acc = acc + _dot(late_o[g - (8 - LATE)], w_out(g))
    yb[pl.ds(2 * NSEG, 2)] = acc.astype(BF16).reshape(2, 16, D)
    b_out(NSEG - 1, 1).start()
    wait_for(ya.at[pl.ds(0, 4096)], sem_a)
    b_out(0, NSEG).wait()


def _forward(A_x, A_w_r, A_w_i, B_x, B_mem0, B_Wq, B_Wk, B_Wv, B_Wo):
    in_hbm = pl.BlockSpec(memory_space=pl.ANY)
    out = pl.pallas_call(
        _kernel,
        out_shape=jax.ShapeDtypeStruct((S // 16, 16, 2 * D), BF16),
        in_specs=[in_hbm] * 13,
        out_specs=in_hbm,
        scratch_shapes=[
            pltpu.VMEM((16, 8, 128), F32),
            pltpu.VMEM((2, 4, 2, 64, D), U32),
            pltpu.VMEM((D // 4, S), U32),
            pltpu.VMEM((D // 4, S), U32),
            pltpu.VMEM((5 * 64, 128), U32),
            pltpu.VMEM((32 * 64, 128), U32),
            pltpu.VMEM((NYQ + 256, 128), F32),
            pltpu.VMEM((ZERO + 32, 128), U32),
            pltpu.VMEM((4096 + 32, 128), U32),
            pltpu.VMEM((PAIRS, D + 32, 128), U32),
            pltpu.VMEM((7, 2 * NSEG, D // 2), U32),
            pltpu.VMEM((4, H * DH // 2, 128), U32),
            pltpu.VMEM((NSEG, 8, D), BF16),
            pltpu.VMEM((NSEG, SEG - 8, D), BF16),
            pltpu.VMEM((3 * H * 8 * NSEG, DH), F32),
            pltpu.VMEM((2 * NSEG + 2, 16, D), BF16),
            pltpu.VMEM((M, D), BF16),
            pltpu.VMEM((1, S), BF16),
            pltpu.VMEM((1, S), BF16),
            pltpu.SMEM((128,), jnp.int32),
            pltpu.SemaphoreType.DMA((10 + sum(p[2] for p in PHASES),)),
        ],
        compiler_params=pltpu.CompilerParams(vmem_limit_bytes=100 * 1024 * 1024),
    )(A_x.reshape(S // 32, 32, D), A_w_r.T, A_w_i.T, B_x.reshape(NSEG, SEG, D), B_mem0.reshape(M, D),
      B_Wq, B_Wk, B_Wv, B_Wo.reshape(H * DH, D), _FD, _G, _TURNS, _INDICES)
    return out.reshape(1, S, 2 * D)


@jax.jit
def pallas_concat_heads__spectral_gfnet__memory_aug_recurrent_mem_tr__prompt_kernel(
    A_x: jax.Array,
    A_w_r: jax.Array,
    A_w_i: jax.Array,
    B_x: jax.Array,
    B_mem0: jax.Array,
    B_Wq: jax.Array,
    B_Wk: jax.Array,
    B_Wv: jax.Array,
    B_Wo: jax.Array,
    B_seg_len: jax.Array,
):
    del B_seg_len
    return _forward(A_x, A_w_r, A_w_i, B_x, B_mem0, B_Wq, B_Wk, B_Wv, B_Wo)
```

```python
import jax
import jax.numpy as jnp
import numpy as np
from jax import lax
import jax.experimental.pallas as pl
import jax.experimental.pallas.tpu as pltpu

F32, BF16, U32 = jnp.float32, jnp.bfloat16, jnp.uint32
NN = (((1,), (0,)), ((), ()))
NT = (((1,), (1,)), ((), ()))

S, D = 2048, 512
M, SEG, H, DH = 8, 32, 32, 128
L = M + SEG
NSEG = S // SEG
LOG2E = 1.4426950408889634

STEPS = 8
LATE = 3
PAIRS = 3 * H // 2
PHASES = ((0, 2, 1), (2, 4, 3), (14, 5, 2), (24, 12, 2))
ORDER_FORWARD = (
    "PPOOPOOOTTOOTOTPTOOTOOOTTPTTTTOOOPPPTTPPPPTPTPPPPPPPPSPPSPSPPSPPPSPSPPSPPPSPPSPPSPPPSPSPPPSPSPSPPPPP"
    "SPSPSPPPPPPPPPPPPPPP"
)
ORDER_FILTER = (
    "PPFPFPFPPFPFPPFPPFPFPPFPPFPPFPPFPFPFPPPFPPFPPPFPFPFPFPPFPPFPPFPPFPPFPFPPFPFPPPFPPFPFPFPFPPFPPPFPFPPP"
    "PFPFPFPPFPFPPPFPFPFPPPFPFPPFPPFPPPFPFPFPFPPFPFPPPFPPFPFPPPFPFPPFPFPPFPPFPPFPFPPFPPFPFPPFPPFPPFPPFPPF"
    "PPFPFPFPPPPFPFPFPFPFPPFPPPFPFPPFPPFPPFPPFPFPPPFPFPFPPFPPFPPFPPFP"
)
SPEC = 3 * H * D // 2
NYQ = 16 * 512
ZERO = SPEC + NYQ + 256


def _dft_constants():
    d = np.arange(128)
    j = (8 * np.arange(8)[:, None] + np.array([0, 4, 1, 5, 2, 6, 3, 7])[None, :]).reshape(-1)

    def cos_sin(r):
        ang = 2 * np.pi * (np.outer(4 * j + r, d) % D) / D
        return np.cos(ang), np.sin(ang)

    (c0, s0), (c1, s1), (c2, s2), (c3, s3) = [cos_sin(r) for r in range(4)]
    f0 = np.concatenate([c0, -s0])
    f0[64] = 1.0 - 2.0 * (d % 2)
    row = np.arange(128)
    cos, sin = np.concatenate([c1, c3])[:, :64], np.concatenate([s1, s3])[:, :64]
    sign = np.where(row < 64, -1.0, 1.0)[:, None]
    real, imag = np.concatenate([cos, sign * sin], axis=1), np.concatenate([-sin, sign * cos], axis=1)[row ^ 2]
    own = (((row & 2) == 0) == (row < 64))[:, None]
    fd = np.stack([f0, np.concatenate([c2, -s2]), np.where(own, real, imag), np.where(own, imag, real),
                   np.concatenate([-s2, c2])])
    i, u, half, sigma, t1, f1 = np.ix_(*[np.arange(n) for n in (2, 4, 2, 2, 64, 64)])
    ang = 2 * np.pi * (((32 * t1 + 16 * sigma + 4 * u + 2 * i + half) * f1) % S) / S
    gr, gi = np.cos(ang), -np.sin(ang)
    g = np.concatenate([np.concatenate([gr, gi], axis=-1), np.concatenate([-gi, gr], axis=-1)], axis=-2)
    ang = 2 * np.pi * np.arange(16)[:, None, None] / 32
    low = np.arange(128)[None, None, :] < 64
    turns = np.concatenate([np.cos(ang) * np.ones_like(low), np.where(low, -np.sin(ang), np.sin(ang)),
                            np.zeros((16, 6, 128))], axis=1)

    def words(a):
        bits = a.astype(np.float32).astype(BF16).view(np.uint16).astype(np.uint32).reshape(-1, 128)
        return bits[0::2] | (bits[1::2] << 16)

    return words(fd), words(g), turns.astype(np.float32)


_FD, _G, _TURNS = _dft_constants()
_INDICES = np.arange(128, dtype=np.int32) ** 2
_C8, _S8, _R2 = float(np.cos(np.pi / 8)), float(np.sin(np.pi / 8)), float(np.sqrt(0.5))

_PRODUCTS = (
    (((0, 0), (1, 1), 1), ((0, 0), (1, 1), 1), (((0, 0), 1), ((1, 1), 1))),
    (((1, 0), (1, 1), 1), ((0, 0),), (((1, 0), 1), ((1, 1), -1))),
    (((1, 1),), ((1, 0), (0, 0), -1), (((0, 0), 1), ((1, 0), 1))),
    (((0, 0), (0, 1), 1), ((1, 1),), (((0, 0), -1), ((0, 1), 1))),
    (((0, 1), (1, 1), -1), ((1, 0), (1, 1), 1), (((0, 0), 1),)),
    (((0, 0),), ((0, 1), (1, 1), -1), (((0, 1), 1), ((1, 1), 1))),
    (((1, 0), (0, 0), -1), ((0, 0), (0, 1), 1), (((1, 1), 1),)),
)


def _dot(a, b, dims=NN):
    return lax.dot_general(a, b, dims, preferred_element_type=F32)


def _radix4(a, b, c, d, sign):
    t0 = (a[0] + c[0], a[1] + c[1])
    t1 = (a[0] - c[0], a[1] - c[1])
    t2 = (b[0] + d[0], b[1] + d[1])
    t3 = (b[0] - d[0], b[1] - d[1])
    y0 = (t0[0] + t2[0], t0[1] + t2[1])
    y2 = (t0[0] - t2[0], t0[1] - t2[1])
    ya = (t1[0] + t3[1], t1[1] - t3[0])
    yb = (t1[0] - t3[1], t1[1] + t3[0])
    return (y0, ya, y2, yb) if sign < 0 else (y0, yb, y2, ya)


def _twiddle16(z, e):
    re, im = z
    if e == 0:
        return z
    if e == 4:
        return -im, re
    if e == 2:
        return (re - im) * _R2, (im + re) * _R2
    if e == 6:
        return (re + im) * (-_R2), (re - im) * _R2
    c, s = {1: (_C8, _S8), 3: (_S8, _C8), 9: (-_C8, -_S8)}[e]
    return re * c - im * s, im * c + re * s


def _lo(w):
    return pltpu.bitcast(w << 16, F32)


def _hi(w):
    return pltpu.bitcast(w & np.uint32(0xFFFF0000), F32)


def _pack(even, odd):
    return (even >> 16) | (odd & np.uint32(0xFFFF0000))


def _kernel(ax_hbm, wr_hbm, wi_hbm, bx_hbm, mem_hbm, wq_hbm, wk_hbm, wv_hbm, wo_hbm, fd_hbm, g_hbm, turns_hbm,
            idx_hbm, out_hbm,
            turns, ax, wr, wi, fd, gt, ybuf, work, ya, raw, xs, wo, xpre, xrest, pre, yb, mem0, wr_last, wi_last, idx,
            sems):
    ax32 = ax_hbm.bitcast(U32)
    wo32 = wo_hbm.bitcast(U32)
    out32 = out_hbm.bitcast(U32)
    w32 = [w.bitcast(U32) for w in (wq_hbm, wk_hbm, wv_hbm)]

    sem_phase = [1 + sum(p[2] for p in PHASES[:n]) for n in range(5)]
    sem_fd, sem_filter, sem_rest, sem_a, sem_b, sem_x, sem_g = [sem_phase[4] + n for n in (0, 1, 2, 3, 4, 5, 7)]

    def pairs(phase, i):
        first, count, _ = PHASES[phase]
        return [(w32[p // 16].at[:, p % 16, :], raw.at[p, pl.ds(0, D)], sem_phase[phase] + i)
                for p in range(first + count * i, first + count * (i + 1))]

    def filters(src, dst, last):
        return [(src.at[pl.ds(0, D // 2)].bitcast(U32), dst, sem_filter), (src.at[pl.ds(D // 2, 1)], last, sem_filter)]

    plan = [(idx_hbm, idx, 0), (bx_hbm.at[:, pl.ds(0, 8), :], xpre, 0)] + pairs(0, 0)
    for i in range(PHASES[1][2]):
        plan += pairs(1, i)
    plan += [(fd_hbm, fd, sem_fd)]
    for i in range(2):
        plan += pairs(2, i)
        plan += [(ax32.at[:, 8 * sigma + 2 * u + i, :], ax.at[i, u, sigma], sem_x + i)
                 for u in range(4) for sigma in range(2)]
        plan += [(g_hbm.at[pl.ds(1024 * i, 1024)], gt.at[pl.ds(1024 * i, 1024)], sem_g + i)]
    plan += filters(wr_hbm, wr, wr_last) + filters(wi_hbm, wi, wi_last)
    for i in range(PHASES[3][2]):
        plan += pairs(3, i)
    plan += [(turns_hbm, turns, sem_rest), (mem_hbm, mem0, sem_rest),
             (bx_hbm.at[:, pl.ds(8, SEG - 8), :], xrest, sem_rest)]
    plan += [(wo32.at[:, pl.ds(128 * j, 128)], wo.at[j], sem_rest) for j in range(4)]
    for src, dst, sem in plan:
        pltpu.make_async_copy(src, dst, sems.at[sem]).start()

    def wait(sem):
        for src, dst, n in plan:
            if n == sem:
                pltpu.make_async_copy(src, dst, sems.at[sem]).wait()

    def wait_for(dst, sem):
        pltpu.make_async_copy(dst, dst, sems.at[sem]).wait()

    sub = lax.broadcasted_iota(jnp.int32, (8, 128), 0)
    lane = lax.broadcasted_iota(jnp.int32, (264, 128), 1)
    low = lane < 64
    row0 = sub == 0

    def rows(base, off, n):
        return pl.ds((base if isinstance(base, int) else pl.multiple_of(base, 32)) + off, n)

    def pinned(base, off, n):
        return rows(idx[0] + base, off, n)

    work[pl.ds(ZERO, 8), :] = jnp.zeros((8, 128), U32)

    def after_stores(words):
        return jnp.concatenate([words[:8] | work[pinned(ZERO, 0, 8), :], words[8:]], axis=0)

    def get(where):
        return pltpu.bitcast(work[where, :], F32)

    def put(where, v):
        work[where, :] = pltpu.bitcast(v, U32)

    fw = {}

    def table(n):
        return pltpu.bitcast(fd[pl.ds(64 * n, 64), :], BF16)

    def by_group(v):
        return jnp.concatenate([v[64 * blk + 8 * jg:64 * blk + 8 * jg + 8] for jg in range(8) for blk in range(4)], 0)

    def by_block(v):
        return jnp.concatenate([v[32 * jg + 8 * blk:32 * jg + 8 * blk + 8] for blk in range(4) for jg in range(8)], 0)

    def a_features(i, u, n):
        if n == 0:
            words = [jnp.concatenate([ax[i, u, sigma, :, 128 * j:128 * (j + 1)] for sigma in range(2)], axis=0)
                     for j in range(4)]
            x = [jnp.concatenate([_lo(w), _hi(w)], axis=0) for w in words]
            a0, a1, b0, b1 = x[0] + x[2], x[1] + x[3], x[0] - x[2], x[1] - x[3]
            base = jnp.where(low[:256], b0, pltpu.roll(b1, 64, 1))
            t = jnp.where(low[:256], pltpu.roll(b0 - b1, 64, 1), b0 + b1) * _R2
            fw[u] = [v.astype(BF16) for v in (a0 + a1, a0 - a1, base + t, base - t)]
        fw[u][n] = _dot(table(n), fw[u][n], NT)

    def a_time(i, u, half, sigma):
        if half == 0 and sigma == 0:
            e0, e2, qa, qb = fw[u]
            first = jnp.concatenate([(sub & 2) == 0] * 2, axis=1)
            re, im = [], []
            for r in range(0, 128, 8):
                x, y = (qa[r:r + 8], qb[r:r + 8]) if r < 64 else (qb[r:r + 8], qa[r:r + 8])
                re.append(jnp.where(first, x, y))
                t = jnp.where(first, y, x)
                im.append(jnp.where(first, pltpu.roll(t, 6, 0), pltpu.roll(t, 2, 0)))
            nyq = e0[64:72]
            fw[u] = (jnp.concatenate([e0[:64], e2[:64]] + re + [nyq], axis=0),
                     jnp.concatenate([jnp.where(jnp.concatenate([row0, row0], axis=1), 0.0, nyq), e0[72:], e2[64:]]
                                     + im + [jnp.zeros_like(nyq)], axis=0))
        g = pltpu.bitcast(gt[rows(1024 * i, 256 * u + 128 * half + 64 * sigma, 64), :], BF16)
        if sigma == 0:
            xr, xi = [v[:, 128 * half:128 * (half + 1)] for v in fw[u]]
            xi = pltpu.roll(xi, 64, 1)
            fw["odd"] = jnp.where(low, xi, xr)
            fw["even"] = _dot(jnp.where(low, xr, xi), g)
            return
        odd = _dot(fw["odd"], jnp.concatenate([g[64:], g[:64]], axis=0))
        total, diff = fw["even"] + odd, fw["even"] - odd
        c, s = [jnp.where(i == 0, f(2 * np.pi * (4 * u + half) / 32), f(2 * np.pi * (4 * u + half + 2) / 32)).astype(F32)
                for f in (np.cos, np.sin)]
        other = pltpu.roll(diff, 64, 1)
        for d, y in enumerate((jnp.where(low, total, c * other + s * diff),
                               jnp.where(low, pltpu.roll(total, 64, 1), c * diff - s * other))):
            ybuf[rows(1024 * i, 2048 * u + 512 * half + 256 * d, 256), :] = by_group(y[:256])
            ybuf[rows(32 * i, NYQ + 64 * u + 16 * half + 8 * d, 8), :] = y[256:]

    def a_spread(i, half, jg):
        tw = [[jnp.where(i == 0, f(2 * np.pi * half * k / 16), f(2 * np.pi * (2 + half) * k / 16)).astype(F32)
               for f in (np.cos, np.sin)] for k in range(4)]
        if jg == 8:
            todo = [[(32 * i, NYQ + 64 * u + 16 * half, 8) for u in range(4)]]
        else:
            todo = [[(1024 * i, 2048 * u + 512 * half + 32 * jg + 8 * blk, 256) for u in range(4)] for blk in range(4)]
        for slots in todo:
            x = _radix4(*[(ybuf[pinned(b, o, 8), :], ybuf[pinned(b, o + d, 8), :]) for b, o, d in slots], -1)
            for k, ((b, o, d), (re, im)) in enumerate(zip(slots, x)):
                if k > 0:
                    c, s = tw[k]
                    re, im = re * c + im * s, im * c - re * s
                put(rows(b, SPEC + o, 8), re)
                put(rows(b, SPEC + o + d, 8), im)

    def weight(i, jg, blk, f):
        cols = slice(128 * f, 128 * (f + 1))
        if blk == 4:
            return tuple(jnp.broadcast_to(r[:, cols].astype(F32) * 0.5, (8, 128)) for r in (wr_last, wi_last))
        out = []
        for r in (wr, wi):
            v = r[rows(64 * i, 16 * jg, 16), cols]
            if blk % 2 == 0:
                v = jnp.where(sub % 2 == 0, v[:8], pltpu.roll(v[8:], 1, 0))
            else:
                v = jnp.where(sub % 2 == 0, pltpu.roll(v[:8], 7, 0), v[8:])
            v = _lo(v) if blk < 2 else _hi(v)
            if blk == 0 and jg == 0:
                v = v * jnp.where(jnp.logical_and(row0, i == 0), 0.5, 1.0).astype(F32)
            out.append(v)
        return tuple(out)

    def slot(jg, blk, s):
        if blk == 4:
            return SPEC + NYQ + 16 * s, SPEC + NYQ + 16 * s + 8
        return SPEC + 512 * s + 32 * jg + 8 * blk, SPEC + 512 * s + 256 + 32 * jg + 8 * blk

    def a_filter(i, jg, blk, t):
        slots = [slot(jg, blk, 4 * t + u) for u in range(4)]
        x = _radix4(*[tuple(get(pinned(128 * i, r, 8)) for r in ri) for ri in slots], -1)
        w = [weight(i, jg, blk, t + 4 * k) for k in range(4)]
        x = [(v[0] * u[0] - v[1] * u[1], v[0] * u[1] + v[1] * u[0]) for v, u in zip(x, w)]
        for n, (ri, v) in enumerate(zip(slots, _radix4(*x, +1))):
            v = _twiddle16(v, t * n)
            put(rows(128 * i, ri[0], 8), v[0])
            put(rows(128 * i, ri[1], 8), v[1])

    def a_gather(i, jg, blk, ts):
        todo = [[slot(jg, blk, 4 * u + t) for u in range(4)] for t in ts]
        values = [[tuple(get(pinned(128 * i, r, 8)) for r in ri) for ri in slots] for slots in todo]
        for slots, x in zip(todo, values):
            for ri, v in zip(slots, _radix4(*x, +1)):
                put(rows(128 * i, ri[0], 8), v[0])
                put(rows(128 * i, ri[1], 8), v[1])

    def filter_work(i, jg, blk):
        return [(a_filter, (i, jg, blk, t)) for t in range(4)] + [(a_gather, (i, jg, blk, ts)) for ts in ((0, 1), (2, 3))]

    def a_inverse_time(c):
        zr, zi = [], []
        for half in range(2):
            ur, ui = [jnp.concatenate([by_block(get(rows(1024 * c, SPEC + 512 * half + 256 * d, 256))),
                                       get(rows(32 * c, SPEC + NYQ + 16 * half + 8 * d, 8))], axis=0)
                      for d in range(2)]
            co, si = turns[2 * c + half, 0:1], turns[2 * c + half, 1:2]
            moved = pltpu.roll(ui, 64, 1)
            base = jnp.where(low, ur, moved)
            t = co * jnp.where(low, pltpu.roll(ur, 64, 1), ui) + si * jnp.where(low, moved, ur)
            for sigma, v in enumerate((base + t, base - t)):
                g = pltpu.bitcast(gt[rows(1024 * (c % 2) + 256 * (c // 2), 128 * half + 64 * sigma, 64), :], BF16)
                k = _dot(g, v[:256].astype(BF16), NT)
                nyq = jnp.sum(g[:64].astype(F32) * v[256:257], axis=1, keepdims=True)
                zr.append(k[:64])
                zi.append(jnp.concatenate([jnp.where(lane[:64] == 0, nyq, k[64:, :128]), k[64:, 128:]], axis=1))
        return jnp.concatenate(zr, axis=0), jnp.concatenate(zi, axis=0)

    def a_inverse_features(c, zr, zi):
        lo = low[:256]
        rot = pltpu.roll(zi[:, :128], 64, 1)
        u0 = _dot(jnp.where(lo, zr[:, :128], rot), table(0))
        u2 = _dot(jnp.where(lo, rot, zr[:, :128]), table(4))
        zr, zi = zr[:, 128:], zi[:, 128:]
        first = (lane[:256] & 2) == 0
        own = first == lo
        zi = jnp.where(first, pltpu.roll(zi, 126, 1), pltpu.roll(zi, 2, 1))
        wa, wb = _dot(jnp.where(own, zr, zi), table(2)), _dot(jnp.where(own, zi, zr), table(3))
        total, diff = wa + wb, wa - wb
        other = pltpu.roll(diff, 64, 1)
        v0 = jnp.where(lo, total, (other + diff) * _R2)
        v1 = jnp.where(lo, pltpu.roll(total, 64, 1), (diff - other) * _R2)
        e0, e1 = u0 + u2, u0 - u2
        for j, y in enumerate((e0 + v0, e1 + v1, e0 - v0, e1 - v1)):
            y = y * (2.0 / (S * D))
            y = pltpu.bitcast(y.astype(BF16).astype(F32), U32)
            y = _pack(y[:128], y[128:])
            for sigma in range(2):
                ya[c, j, pl.ds(sigma, 64, stride=2), :] = y[64 * sigma:64 * (sigma + 1)]

    part = {}

    def combine(spec, block):
        a, b = block(*spec[0]), block(*spec[1])
        return (a + b if spec[2] > 0 else a - b).astype(BF16)

    def early(p, n, mc):
        _, right, uses = _PRODUCTS[n]
        x = xs[n, (pinned if isinstance(p, int) else rows)(0, 64 * mc, 64), :]
        if mc == 1:
            x = jnp.concatenate([after_stores(x[:, :128]), x[:, 128:]], axis=1)
        elif len(right) > 1:
            def block(r, c):
                words = raw[p, pl.ds(D // 2 * r, D // 2), :]
                return (_lo, _hi)[c](after_stores(words) if (r, c) == right[0] else words)

            part["w"] = combine(right, block)
        else:
            r, c = right[0]
            even, odd = [raw[p, pl.ds(D // 2 * r + t, D // 4, stride=2), :] for t in range(2)]
            plain = (even & np.uint32(0xFFFF)) | (odd << 16), _pack(even, odd)
            part["w"] = pltpu.bitcast(after_stores(plain[c]), BF16)
            for h in range(2):
                work[rows(p * D, h * (D // 2) + r * (D // 4), D // 4), :] = plain[h]
        prod = _dot(pltpu.bitcast(x, BF16), part["w"])
        for key, sign in uses:
            total, count = part.pop((key, mc), (None, 0))
            total = prod if total is None else (total + prod if sign > 0 else total - prod)
            if count + 1 == (4 if key[0] == key[1] else 2):
                pre[rows(p * 16 * NSEG, key[1] * 8 * NSEG + 4 * NSEG * key[0] + 128 * mc, 128), :] = total
            else:
                part[key, mc] = total, count + 1

    def early_work(phase, i):
        first, count, _ = PHASES[phase]
        wait_for(raw.at[pl.ds(first + count * i, count), pl.ds(0, D)], sem_phase[phase] + i)
        return [(early, (first + count * i + u, n, mc)) for u in range(count) for n in range(7) for mc in range(2)]

    def run(order, **queues):
        for name in order:
            fn, args = queues[name].pop(0)
            fn(*args)
        assert not any(queues.values())

    def plain_phase(phase, i):
        todo = early_work(phase, i)
        run("P" * len(todo), P=todo)

    def forward_phase(i):
        wait_for(ax.at[i], sem_x + i)
        wait_for(gt.at[rows(1024 * i, 0, 1024)], sem_g + i)
        run(ORDER_FORWARD, P=early_work(2, i),
            O=[(a_features, (i, u, n)) for u in range(4) for n in range(4)],
            T=[(a_time, (i, u, half, sigma)) for u in range(4) for half in range(2) for sigma in range(2)],
            S=[(a_spread, (i, half, jg)) for jg in range(9) for half in range(2)])

    def filter_phase(i):
        run(ORDER_FILTER, P=early_work(3, i), F=[w for jg in range(4) for blk in range(4) for w in filter_work(i, jg, blk)])

    wait(0)
    xp = xpre[...].reshape(8 * NSEG, D)

    def block_of_x(r, c):
        return xp[256 * r:256 * (r + 1), 256 * c:256 * (c + 1)]

    for n, (left, _, _) in enumerate(_PRODUCTS):
        x = block_of_x(*left[0]) if len(left) == 1 else combine(left, lambda r, c: block_of_x(r, c).astype(F32))
        xs[n] = pltpu.bitcast(x, U32)
    plain_phase(0, 0)
    pl.loop(0, PHASES[1][2])(lambda i: plain_phase(1, i))
    wait(sem_fd)
    pl.loop(0, 2)(forward_phase)
    wait(sem_filter)
    run("F" * 6, F=filter_work(0, 0, 4))
    pl.loop(0, 2)(filter_phase)
    wait(sem_rest)

    row = lax.broadcasted_iota(jnp.int32, (L, L), 0)
    col = lax.broadcasted_iota(jnp.int32, (L, L), 1)
    mask = (row >= SEG) | (col >= SEG) | (row >= col)
    scale = DH ** -0.5

    def w_in(i, g):
        return jnp.concatenate(
            [pltpu.bitcast(work[pl.ds((i * H + 4 * g + j) * (D // 2), D // 2), :], BF16) for j in range(4)], axis=1)

    def w_out(g):
        return jnp.concatenate([pltpu.bitcast(wo[j, 256 * g:256 * (g + 1)], BF16) for j in range(4)], axis=1)

    def keep(s, out):
        words = pltpu.bitcast(out.astype(BF16), U32)
        for j in range(4):
            yb[j, pl.ds(2 * s, 2)] = words[:, 128 * j:128 * (j + 1)].reshape(2, 8, 128)

    def step(s, carry, c=None):
        mem, late_o, late_acc = carry
        h = jnp.concatenate([xrest[s].astype(F32), mem], axis=0).astype(BF16)
        st = {"late": late_acc}

        def project(i, g):
            known = [pre[pl.ds(pl.multiple_of(s * 8, 8) + (i * H + 4 * g + j) * 8 * NSEG, 8), :] for j in range(4)]
            st[i, g] = jnp.concatenate([jnp.concatenate(known, axis=1), _dot(h, w_in(i, g))], axis=0)

        def softmax(g):
            ps = []
            for j in range(4):
                cols = slice(DH * j, DH * (j + 1))
                sc = _dot(st[0, g][:, cols], st[1, g][:, cols], NT)
                sc = jnp.where(mask, sc * (scale * LOG2E), -1e9 * LOG2E)
                e = jnp.exp2(sc - jnp.max(sc, axis=1, keepdims=True))
                total = jnp.sum(e, axis=1, keepdims=True)
                r = pltpu.reciprocal(total, approx=True)
                ps.append((e, r * (2.0 - total * r)))
            st["p", g] = ps

        def mix_rows(g, which):
            v = st[2, g].astype(BF16)
            return jnp.concatenate([_dot(e[which], v[:, DH * j:DH * (j + 1)]) * r[which]
                                    for j, (e, r) in enumerate(st["p", g])], axis=1)

        def mix(g):
            if g >= 8 - LATE:
                st["o", g] = jnp.concatenate([mix_rows(g, slice(SEG, L)), late_o[g - (8 - LATE)]], axis=0)
            else:
                o = mix_rows(g, slice(0, L))
                st["o", g] = jnp.concatenate([o[SEG:], o[:SEG]], axis=0)

        def output(g):
            r = _dot(st["o", g], w_out(g))
            st["mem"] = r[:M] if g == 0 else st["mem"] + r[:M]
            key = "late" if g >= 8 - LATE else "tokens"
            st[key] = r[M:] if g == 0 else st[key] + r[M:]

        for g in range(8):
            project(1, g)
            project(0, g)
            if g > 0:
                mix(g - 1)
            project(2, g)
            softmax(g)
        if c is not None:
            z = a_inverse_time(c)
        for g in range(8):
            output(g)
            if g == 1:
                mix(7)
            if g == 3 and c is not None:
                a_inverse_features(c, *z)
        late_o = tuple(mix_rows(g, slice(0, SEG)) for g in range(8 - LATE, 8))
        keep(s, st["late"])
        return st["mem"], late_o, st["tokens"]

    def b_out(first, n):
        for j in range(4):
            pltpu.make_async_copy(yb.at[j, pl.ds(2 * first + 2, 2 * n)],
                                  out32.at[pl.ds(2 * first, 2 * n), :, pl.ds(D + 128 * j, 128)], sems.at[sem_b]).start()

    def block(i, carry):
        for u in range(STEPS):
            carry = step(i * STEPS + u, carry, i if u == STEPS - 1 else None)
            if u == 0:
                pl.when(i > 0)(lambda: b_out(i * STEPS - 2, 2))
            if u == STEPS - 2:
                b_out(i * STEPS, STEPS - 2)
        for j in range(4):
            pltpu.make_async_copy(
                ya.at[i, j, pl.ds(0, 128)], out32.at[:, i, pl.ds(128 * j, 128)], sems.at[sem_a]).start()
        return carry

    zeros = jnp.zeros((SEG, D), F32)
    _, late_o, acc = lax.fori_loop(0, NSEG // STEPS, block, (mem0[...].astype(F32), (zeros,) * LATE, zeros))
    for g in range(8 - LATE, 8):
        acc = acc + _dot(late_o[g - (8 - LATE)], w_out(g))
    keep(NSEG, acc)
    b_out(NSEG - 2, 2)
    wait_for(out32.at[:, :, pl.ds(0, D)], sem_a)
    wait_for(out32.at[:, :, pl.ds(D, D)], sem_b)


def _forward(A_x, A_w_r, A_w_i, B_x, B_mem0, B_Wq, B_Wk, B_Wv, B_Wo):
    in_hbm = pl.BlockSpec(memory_space=pl.ANY)
    out = pl.pallas_call(
        _kernel,
        out_shape=jax.ShapeDtypeStruct((S // 16, 16, 2 * D), BF16),
        in_specs=[in_hbm] * 13,
        out_specs=in_hbm,
        scratch_shapes=[
            pltpu.VMEM((16, 8, 128), F32),
            pltpu.VMEM((2, 4, 2, 64, D), U32),
            pltpu.VMEM((D // 4, S), U32),
            pltpu.VMEM((D // 4, S), U32),
            pltpu.VMEM((5 * 64, 128), U32),
            pltpu.VMEM((32 * 64, 128), U32),
            pltpu.VMEM((NYQ + 256, 128), F32),
            pltpu.VMEM((ZERO + 32, 128), U32),
            pltpu.VMEM((8, 4, 128 + 32, 128), U32),
            pltpu.VMEM((PAIRS, D + 32, 128), U32),
            pltpu.VMEM((7, 2 * NSEG, D // 2), U32),
            pltpu.VMEM((4, H * DH // 2, 128), U32),
            pltpu.VMEM((NSEG, 8, D), BF16),
            pltpu.VMEM((NSEG, SEG - 8, D), BF16),
            pltpu.VMEM((3 * H * 8 * NSEG, DH), F32),
            pltpu.VMEM((4, 2 * NSEG + 4, 8, 128), U32),
            pltpu.VMEM((M, D), BF16),
            pltpu.VMEM((1, S), BF16),
            pltpu.VMEM((1, S), BF16),
            pltpu.SMEM((128,), jnp.int32),
            pltpu.SemaphoreType.DMA((10 + sum(p[2] for p in PHASES),)),
        ],
        compiler_params=pltpu.CompilerParams(vmem_limit_bytes=100 * 1024 * 1024),
    )(A_x.reshape(S // 32, 32, D), A_w_r.T, A_w_i.T, B_x.reshape(NSEG, SEG, D), B_mem0.reshape(M, D),
      B_Wq, B_Wk, B_Wv, B_Wo.reshape(H * DH, D), _FD, _G, _TURNS, _INDICES)
    return out.reshape(1, S, 2 * D)


@jax.jit
def pallas_concat_heads__spectral_gfnet__memory_aug_recurrent_mem_tr__prompt_kernel(
    A_x: jax.Array,
    A_w_r: jax.Array,
    A_w_i: jax.Array,
    B_x: jax.Array,
    B_mem0: jax.Array,
    B_Wq: jax.Array,
    B_Wk: jax.Array,
    B_Wv: jax.Array,
    B_Wo: jax.Array,
    B_seg_len: jax.Array,
):
    del B_seg_len
    return _forward(A_x, A_w_r, A_w_i, B_x, B_mem0, B_Wq, B_Wk, B_Wv, B_Wo)
```
